```python
import os as _os
_os.environ.setdefault("JAX_PLATFORMS", "cpu")
import jax
import jax.numpy as jnp

def _softmax(x, axis=-1):
    return jax.nn.softmax(x, axis=axis)
def _gelu(x):
    return jax.nn.gelu(x, approximate=True)
def _silu(x):
    return jax.nn.silu(x)
def _sigmoid(x):
    return jax.nn.sigmoid(x)
def _layernorm(x, axis=-1, eps=1e-5):
    m = jnp.mean(x, axis=axis, keepdims=True)
    v = jnp.var(x, axis=axis, keepdims=True)
    return (x - m) / jnp.sqrt(v + eps)
def _scatter_add(tgt, idx, src, axis=0):
    return tgt.at[idx].add(src)
def _segment_sum(src, seg, n):
    return jax.ops.segment_sum(src, seg, n)
class _Rng:
    def __init__(self, key):
        self._k = key
    def _next(self):
        self._k, sub = jax.random.split(self._k)
        return sub
    def normal(self, shape):
        return jax.random.normal(self._next(), shape, dtype=jnp.bfloat16)
    def randint(self, lo, hi, shape):
        return jax.random.randint(self._next(), shape, lo, hi, dtype=jnp.int32)
    def uniform(self, shape, lo=0.0, hi=1.0):
        return jax.random.uniform(self._next(), shape, jnp.bfloat16, lo, hi)
    def permutation(self, n):
        return jax.random.permutation(self._next(), n)


kernel_name = 'concat_heads__gqa_block_cached__gqa_block_cached__near_ridge'

def setup_inputs():
    _rng = _Rng(jax.random.key(int.from_bytes(__import__("os").urandom(4), "little")))
    _w = (lambda a: (lambda t: t.astype(jnp.bfloat16) if jnp.issubdtype(t.dtype, jnp.floating) else t)(jnp.asarray(a)))
    def _A_setup():
        B, Sq, D = 16, 144, 448
        Hq, Hkv, Sk, Dh = 16, 8, 1024, 256
        assert Hq % Hkv == 0, (Hq, Hkv)
        return {
            "x": _w((lambda *s: _rng.normal(s) * 0.8)(B, Sq, D)),
            "k_cache": _w((lambda *s: _rng.normal(s) * 0.8)(B, Hkv, Sk, Dh)),
            "v_cache": _w((lambda *s: _rng.normal(s) * 0.05)(B, Hkv, Sk, Dh)),
            "wq": _w((lambda *s: _rng.normal(s) * 0.8)(D, Hq * Dh) * (D ** -0.5)),
            "wo": _w((lambda *s: _rng.normal(s) * 0.05)(Hq * Dh, D) * ((Hq * Dh) ** -0.5)),
        }
    _A_in = _A_setup()

    def _B_setup():
        B, Sq, D = 16, 144, 448
        Hq, Hkv, Sk, Dh = 16, 8, 1024, 256
        assert Hq % Hkv == 0, (Hq, Hkv)
        return {
            "x": _w((lambda *s: _rng.normal(s) * 0.8)(B, Sq, D)),
            "k_cache": _w((lambda *s: _rng.normal(s) * 0.8)(B, Hkv, Sk, Dh)),
            "v_cache": _w((lambda *s: _rng.normal(s) * 0.05)(B, Hkv, Sk, Dh)),
            "wq": _w((lambda *s: _rng.normal(s) * 0.8)(D, Hq * Dh) * (D ** -0.5)),
            "wo": _w((lambda *s: _rng.normal(s) * 0.05)(Hq * Dh, D) * ((Hq * Dh) ** -0.5)),
        }
    _B_in = _B_setup()

    return {
        "A_x": _A_in["x"],
        "A_k_cache": _A_in["k_cache"],
        "A_v_cache": _A_in["v_cache"],
        "A_wq": _A_in["wq"],
        "A_wo": _A_in["wo"],
        "B_x": _B_in["x"],
        "B_k_cache": _B_in["k_cache"],
        "B_v_cache": _B_in["v_cache"],
        "B_wq": _B_in["wq"],
        "B_wo": _B_in["wo"],
    }

def reference(A_x, A_k_cache, A_v_cache, A_wq, A_wo, B_x, B_k_cache, B_v_cache, B_wq, B_wo):
    def _A_ref(x, k_cache, v_cache, wq, wo):
        B, Sq, D = x.shape
        Hq, Dh = 16, 256
        Hkv = k_cache.shape[1]
        rep = Hq // Hkv
        q = (lambda x, *d: x.transpose(*d))((x @ wq).reshape(B, Sq, Hq, Dh), 0, 2, 1, 3)
        k = jnp.repeat(k_cache, rep, axis=1)
        v = jnp.repeat(v_cache, rep, axis=1)
        scores = jnp.einsum("bhqd,bhkd->bhqk", q, k) * (Dh ** -0.5)
        p = _softmax(scores, axis=-1)
        o = jnp.einsum("bhqk,bhkd->bhqd", p, v)
        return (lambda x, *d: x.transpose(*d))(o, 0, 2, 1, 3).reshape(B, Sq, Hq * Dh) @ wo

    def _B_ref(x, k_cache, v_cache, wq, wo):
        B, Sq, D = x.shape
        Hq, Dh = 16, 256
        Hkv = k_cache.shape[1]
        rep = Hq // Hkv
        q = (lambda x, *d: x.transpose(*d))((x @ wq).reshape(B, Sq, Hq, Dh), 0, 2, 1, 3)
        k = jnp.repeat(k_cache, rep, axis=1)
        v = jnp.repeat(v_cache, rep, axis=1)
        scores = jnp.einsum("bhqd,bhkd->bhqk", q, k) * (Dh ** -0.5)
        p = _softmax(scores, axis=-1)
        o = jnp.einsum("bhqk,bhkd->bhqd", p, v)
        return (lambda x, *d: x.transpose(*d))(o, 0, 2, 1, 3).reshape(B, Sq, Hq * Dh) @ wo

    a = _A_ref(A_x, A_k_cache, A_v_cache, A_wq, A_wo)
    b = _B_ref(B_x, B_k_cache, B_v_cache, B_wq, B_wo)
    return jnp.concatenate([a, b], axis=-1)
```

```python
import functools
import math
import os
import jax
import jax.numpy as jnp
import jax.experimental.pallas as pl
import jax.experimental.pallas.tpu as pltpu

B, SQ, D = 16, 144, 448
HQ, HKV, SK, DH = 16, 8, 1024, 256
REP = HQ // HKV
GW = REP * DH
QSCALE = (DH ** -0.5) * math.log2(math.e)
NT = (((1,), (1,)), ((), ()))
GB = 8
NG = B // GB
GR = GB * SQ
MT = GR // 128
NU = 2 * GB
NIT = NG * HKV
M = B * SQ
R2 = REP * SQ
SPI = int(os.environ.get("SPI", "1"))
CH = int(os.environ.get("CH", "16"))
SPREAD = float(os.environ.get("SPREAD", "0.9"))
RECIP = int(os.environ.get("RECIP", "1"))
XPIECES = (2, 4, 10)
NODMA = int(os.environ.get("NODMA", "0"))
P2N = int(os.environ.get("P2N", "16"))
P1N = int(os.environ.get("P1N", "5"))
f32, bf16 = jnp.float32, jnp.bfloat16


def _kernel(xa, ka, va, wqa, woa, xb, kb, vb, wqb, wob, out_hbm,
            kvbuf, xbuf, wqbuf, wobuf, qbuf, obuf_a, obuf_b, acc, stage,
            kvsem, xsem, wqsem, wosem, osem):
    x_hbm, kv_hbm = (xa, xb), (ka, va, kb, vb)
    wq_hbm, wo_hbm = (wqa, wqb), (woa, wob)
    obufs = (obuf_a, obuf_b)

    def kv_copies(slot, g, h):
        return [pltpu.make_async_copy(kv_hbm[i].at[pl.ds(g * GB, GB), h], kvbuf.at[slot, i], kvsem.at[slot * 4 + i])
                for i in range(4)]

    def wo_copies(slot, h):
        col = h * GW if isinstance(h, int) else pl.multiple_of(h * GW, GW)
        return [pltpu.make_async_copy(wo_hbm[br].at[:, pl.ds(col, GW)], wobuf.at[slot, br], wosem.at[slot * 2 + br])
                for br in range(2)]

    def wq_copy(s):
        br, h = divmod(s, HKV)
        return pltpu.make_async_copy(wq_hbm[br].at[:, pl.ds(h * GW, GW)], wqbuf.at[s], wqsem.at[s])

    xp = []
    r0 = 0
    for n in XPIECES:
        xp.append((r0, n * SQ))
        r0 += n * SQ

    def xa_copy(i):
        r, n = xp[i]
        return pltpu.make_async_copy(x_hbm[0].at[pl.ds(r, n)], xbuf.at[0, pl.ds(r, n)], xsem.at[i])

    def xb_copy():
        return pltpu.make_async_copy(x_hbm[1], xbuf.at[1], xsem.at[len(xp)])

    def out_copy(t, g):
        row = g * GR + t * 128
        return pltpu.make_async_copy(stage.at[pl.ds(t * 128, 128)], out_hbm.at[pl.ds(row, 128)], osem.at[t])

    xa_copy(0).start()
    wq_copy(0).start()

    def q_rows(s, br, r, n):
        q = jnp.dot(xbuf[br, pl.ds(r, n), :], wqbuf[s], preferred_element_type=f32)
        qbuf[s, pl.ds(r, n), :] = (q * QSCALE).astype(bf16)

    xa_copy(1).start()
    wq_copy(0).wait()
    xa_copy(0).wait()
    xa_copy(2).start()
    q_rows(0, 0, *xp[0])
    xa_copy(1).wait()
    for s in range(1, 1 + SPI):
        wq_copy(s).start()
    xb_copy().start()
    q_rows(0, 0, *xp[1])
    xa_copy(2).wait()
    q_rows(0, 0, *xp[2])
    xb_copy().wait()
    for s in range(1 + SPI, 2 * HKV):
        wq_copy(s).start()

    def p1_body(i, carry):
        @pl.when(i == 1)
        def _():
            for c in kv_copies(0, 0, 0):
                c.start()
            for c in wo_copies(0, 0):
                c.start()
        for k in range(SPI):
            s = 1 + i * SPI + k
            pltpu.make_async_copy(wqbuf.at[s], wqbuf.at[s], wqsem.at[s]).wait()
        for k in range(SPI):
            s = 1 + i * SPI + k
            q_rows(s, s // HKV, 0, M)
        return carry

    jax.lax.fori_loop(0, (2 * HKV - 1) // SPI, p1_body, 0)

    def finalize(g):
        for t in range(MT):
            stage[t * 128:(t + 1) * 128, :] = acc[:, t * 128:(t + 1) * 128].T.astype(bf16)
            out_copy(t, g).start()

    def body(it, carry):
        g = it // HKV
        h = it % HKV
        slot = it % 2
        nit = jnp.minimum(it + 1, NIT - 1)
        if not NODMA:
            for c in kv_copies(1 - slot, nit // HKV, nit % HKV):
                c.start()
            for c in wo_copies(1 - slot, nit % HKV):
                c.start()

        @pl.when(it == HKV)
        def _():
            finalize(0)

        if not NODMA:
            for c in kv_copies(slot, g, h):
                c.wait()
            for c in wo_copies(slot, h):
                c.wait()
        first = h == 0
        always = it >= 0

        def qk(u):
            br, j = divmod(u, GB)
            row = pl.multiple_of((g * GB + j) * SQ, 16)
            s_idx = br * HKV + h
            q2 = jnp.concatenate([qbuf[s_idx, pl.ds(row, SQ), 0:DH], qbuf[s_idx, pl.ds(row, SQ), DH:2 * DH]], axis=0)
            return [jax.lax.dot_general(q2, kvbuf[slot, 2 * br, j, c * 256:(c + 1) * 256, :], NT,
                                        preferred_element_type=f32) for c in range(4)]

        def tokens_from(pieces, nrows, n, spread):
            total = len(pieces) * nrows
            out = []
            for c in range(n):
                pos = int(c * spread * total / n)
                pi, r = divmod(pos, nrows)
                r = min((r // 8) * 8, nrows - CH)
                out.append(pieces[pi][r:r + CH, 0:128])
            return out

        def sm(s4, toks):
            ps, rs = [], []
            for c in range(R2 // CH):
                rows = slice(c * CH, (c + 1) * CH)
                s = jnp.concatenate([x[rows, :] for x in s4], axis=1)
                m = jnp.broadcast_to(jnp.max(s, axis=-1, keepdims=True), (CH, 128))
                if toks is not None:
                    m = jnp.where(always, m, toks[c])
                p = jnp.exp2(s - jnp.concatenate([m] * (SK // 128), axis=1))
                l = jnp.sum(p, axis=-1, keepdims=True)
                ps.append(p.astype(bf16))
                if RECIP == 0:
                    rs.append(1.0 / l)
                else:
                    r = pl.reciprocal(l, approx=True)
                    rs.append(r * (2.0 - l * r))
            return jnp.concatenate(ps, axis=0), jnp.concatenate(rs, axis=0)

        def pv(u, p, r):
            br, j = divmod(u, GB)
            o = jnp.dot(p, kvbuf[slot, 2 * br + 1, j], preferred_element_type=f32)
            ob = (o * r).astype(bf16)
            obufs[br][j * SQ:(j + 1) * SQ, 0:DH] = ob[:SQ]
            obufs[br][j * SQ:(j + 1) * SQ, DH:2 * DH] = ob[SQ:]
            return o

        def o_proj(br, t):
            r = jax.lax.dot_general(wobuf[slot, br], obufs[br][t * 128:(t + 1) * 128, :], NT,
                                    preferred_element_type=f32)
            old = acc[br * D:(br + 1) * D, t * 128:(t + 1) * 128]
            acc[br * D:(br + 1) * D, t * 128:(t + 1) * 128] = jnp.where(first, 0.0, old) + r
            return r

        nch = R2 // CH
        pending = []
        s_cur = qk(0)
        last_toks = None
        for u in range(NU):
            br, j = divmod(u, GB)
            if u + 1 < NU:
                s_nxt = qk(u + 1)
                toks = tokens_from(s_nxt, R2, nch, SPREAD)
            else:
                toks = last_toks
            p, r = sm(s_cur, toks)
            ro = None
            if pending:
                ro = o_proj(*pending.pop(0))
            o = pv(u, p, r)
            if u == NU - 2:
                last_toks = tokens_from([ro], D, nch // 2, 1.0) + tokens_from([o], R2, nch - nch // 2, 1.0)
            s_cur = s_nxt
            pending.append((br, j))
            if j == GB - 1:
                pending.append((br, GB))
        for t in pending:
            o_proj(*t)
        return carry

    jax.lax.fori_loop(0, P2N, body, 0)

    if P2N > HKV:
        for t in range(MT):
            out_copy(t, 0).wait()
    finalize(1)
    for c in kv_copies(0 if NODMA else P2N % 2, NG - 1, HKV - 1):
        c.wait()
    for c in wo_copies(0 if NODMA else P2N % 2, HKV - 1):
        c.wait()
    for t in range(MT):
        out_copy(t, NG - 1).wait()


@jax.jit
def pallas_concat_heads__gqa_block_cached__gqa_block_cached__near_ridge_kernel(
    A_x, A_k_cache, A_v_cache, A_wq, A_wo, B_x, B_k_cache, B_v_cache, B_wq, B_wo,
):
    any_spec = pl.BlockSpec(memory_space=pl.ANY)
    scratch = [
        pltpu.VMEM((2, 4, GB, SK, DH), bf16),
        pltpu.VMEM((2, M, D), bf16),
        pltpu.VMEM((2 * HKV, D, GW), bf16),
        pltpu.VMEM((2, 2, D, GW), bf16),
        pltpu.VMEM((2 * HKV, M, GW), bf16),
        pltpu.VMEM((GR, GW), bf16),
        pltpu.VMEM((GR, GW), bf16),
        pltpu.VMEM((2 * D, GR), f32),
        pltpu.VMEM((GR, 2 * D), bf16),
        pltpu.SemaphoreType.DMA((8,)),
        pltpu.SemaphoreType.DMA((len(XPIECES) + 1,)),
        pltpu.SemaphoreType.DMA((2 * HKV,)),
        pltpu.SemaphoreType.DMA((4,)),
        pltpu.SemaphoreType.DMA((MT,)),
    ]
    out = pl.pallas_call(
        _kernel,
        in_specs=[any_spec] * 10,
        out_specs=any_spec,
        out_shape=jax.ShapeDtypeStruct((M, 2 * D), bf16),
        scratch_shapes=scratch,
        compiler_params=pltpu.CompilerParams(vmem_limit_bytes=120 * 1024 * 1024),
    )(A_x.reshape(M, D), A_k_cache, A_v_cache, A_wq, A_wo.T,
      B_x.reshape(M, D), B_k_cache, B_v_cache, B_wq, B_wo.T)
    return out.reshape(B, SQ, 2 * D)
```

```python
import math

import jax
import jax.numpy as jnp
import jax.experimental.pallas as pl
import jax.experimental.pallas.tpu as pltpu

B, SQ, D = 16, 144, 448
HQ, HKV, SK, DH = 16, 8, 1024, 256
REP = HQ // HKV
GW = REP * DH
QSCALE = (DH ** -0.5) * math.log2(math.e)
NT = (((1,), (1,)), ((), ()))
GB = 8
NG = B // GB
GR = GB * SQ
MT = GR // 128
NU = 2 * GB
NIT = NG * HKV
M = B * SQ
R2 = REP * SQ
CA = 384
CH = 8
MARGIN = 400
QB = 2
QPOS = (-1, 0, 2, 4)
XROWS = (128, 336, 688, 1152)
f32, bf16 = jnp.float32, jnp.bfloat16
S_WQ, S_WQB, S_KV, S_WO, S_OUT, S_XB, S_X = 0, 3, 4, 6, 8, 9, 10
NSEM = S_X + len(XROWS)


def _kernel(xa, ka, va, wqa, woa, xb, kb, vb, wqb, wob, out_hbm,
            kvbuf, xbuf_a, xbuf_b, wqbuf_a, wqbuf_b, wobuf, qbuf_a, qbuf_b, obuf_a, obuf_b,
            acc, stage, sems):
    kv_hbm = (ka, va, kb, vb)
    wo_hbm = (woa, wob)
    obufs = (obuf_a, obuf_b)
    last_tile = slice((MT - 1) * 128, MT * 128)

    def wait_all(buf, sem):
        pltpu.make_async_copy(buf, buf, sems.at[sem]).wait()

    def wo_copy(br, slot, h):
        col = h * GW if isinstance(h, int) else pl.multiple_of(h * GW, GW)
        return pltpu.make_async_copy(wo_hbm[br].at[:, pl.ds(col, GW)], wobuf.at[slot, br],
                                     sems.at[S_WO + slot])

    def start_slot(slot, g, h):
        for i in range(4):
            pltpu.make_async_copy(kv_hbm[i].at[pl.ds(g * GB, GB), h], kvbuf.at[slot, i],
                                  sems.at[S_KV + slot]).start()
        for br in range(2):
            wo_copy(br, slot, h).start()

    def wqa_copy(h):
        return pltpu.make_async_copy(wqa.at[:, pl.ds(h * GW, GW)], wqbuf_a.at[h],
                                     sems.at[S_WQ + min(h, 2)])

    xp = []
    r0 = 0
    for n in XROWS:
        xp.append((r0, n))
        r0 += n

    def xa_copy(i):
        r, n = xp[i]
        return pltpu.make_async_copy(xa.at[pl.ds(r, n)], xbuf_a.at[pl.ds(r, n)], sems.at[S_X + i])

    def out_copy(row, br):
        cols = pl.ds(0, CA) if br == 0 else pl.ds(CA, 2 * D - CA)
        return pltpu.make_async_copy(stage.at[pl.ds(row, 128), cols],
                                     out_hbm.at[pl.ds(row, 128), cols], sems.at[S_OUT])

    wqa_copy(0).start()
    for i in range(len(xp)):
        xa_copy(i).start()
    for h in range(1, HKV):
        wqa_copy(h).start()
    pltpu.make_async_copy(xb, xbuf_b, sems.at[S_XB]).start()
    for h in range(HKV):
        pltpu.make_async_copy(wqb.at[:, pl.ds(h * GW, GW)], wqbuf_b.at[h], sems.at[S_WQB]).start()
    start_slot(0, 0, 0)

    def qa_rows(h, r, n):
        q = jnp.dot(xbuf_a[pl.ds(r, n), :], wqbuf_a[h], preferred_element_type=f32)
        qbuf_a[h, pl.ds(r, n), :] = (q * QSCALE).astype(bf16)

    acc[CA:2 * D, last_tile] = jnp.zeros((2 * D - CA, 128), f32)
    wqa_copy(0).wait()
    for i in range(len(xp) - 1):
        xa_copy(i).wait()
        qa_rows(0, *xp[i])
    xa_copy(len(xp) - 1).wait()
    wqa_copy(1).wait()

    def p1_body(i, carry):
        @pl.when(i == 1)
        def _():
            wait_all(wqbuf_a.at[pl.ds(2, HKV - 2)], S_WQ + 2)

        qa_rows(3 * ((i + 1) >> 1), pl.multiple_of(GR * ((i + 1) & 1), GR), GR)
        qa_rows(1 + i + (i >> 1), 0, M)
        return carry

    jax.lax.fori_loop(0, 5, p1_body, 0)
    wait_all(xbuf_b, S_XB)
    wait_all(wqbuf_b, S_WQB)

    def stage_tile(br, t, g, val, cond):
        row = g * GR + t * 128
        if not isinstance(row, int):
            row = pl.multiple_of(row, 128)
        if br == 0:
            stage[pl.ds(row, 128), 0:CA] = val[0:CA].T.astype(bf16)
        else:
            full = jnp.concatenate([acc[CA:D, t * 128:(t + 1) * 128], val], axis=0)
            stage[pl.ds(row, 128), CA:2 * D] = full.T.astype(bf16)
        if cond is None:
            out_copy(row, br).start()
        else:
            @pl.when(cond)
            def _():
                out_copy(row, br).start()

    def body(it, carry):
        g = it >> 3
        h = it & 7
        slot = it & 1
        wait_all(kvbuf.at[slot], S_KV + slot)
        wait_all(wobuf.at[slot], S_WO + slot)
        first = h == 0
        last = h == HKV - 1
        always = it >= 0
        stream = []

        def qb_proj(i):
            n = QB * SQ
            row = pl.multiple_of(g * GR + i * n, 16)
            x = xbuf_b[pl.ds(row, n), :]
            for c in range(4):
                q = jnp.dot(x, wqbuf_b[h, :, c * 128:(c + 1) * 128], preferred_element_type=f32)
                stream.append((q, n))
                qbuf_b[i * n:(i + 1) * n, c * 128:(c + 1) * 128] = (q * QSCALE).astype(bf16)

        def qk(u):
            br, j = divmod(u, GB)
            if br == 0:
                rows = pl.ds(pl.multiple_of((g * GB + j) * SQ, 16), SQ)
                q2 = jnp.concatenate([qbuf_a[h, rows, 0:DH], qbuf_a[h, rows, DH:2 * DH]], axis=0)
            else:
                rows = slice(j * SQ, (j + 1) * SQ)
                q2 = jnp.concatenate([qbuf_b[rows, 0:DH], qbuf_b[rows, DH:2 * DH]], axis=0)
            s4 = [jax.lax.dot_general(q2, kvbuf[slot, 2 * br, j, c * 256:(c + 1) * 256, :], NT,
                                      preferred_element_type=f32) for c in range(4)]
            stream.extend((x, R2) for x in s4)
            return s4, len(stream)

        def tokens(start, n):
            win = stream[start:]
            total = sum(nr for _, nr in win) - MARGIN
            out = []
            for c in range(n):
                pos = c * total // n
                for val, nr in win:
                    if pos < nr:
                        break
                    pos -= nr
                r = min((pos // 8) * 8, nr - CH)
                out.append(val[r:r + CH, 0:128])
            return out

        def softmax(s4, start):
            nch = R2 // CH
            toks = tokens(start, nch)
            ps = []
            for c in range(nch):
                rows = slice(c * CH, (c + 1) * CH)
                tiles = [x[rows, k * 128:(k + 1) * 128] for x in s4 for k in range(2)]
                m = jnp.where(always, tiles[0], toks[c])
                for t in tiles[1:]:
                    m = jnp.maximum(m, t)
                m = jnp.max(m, axis=-1, keepdims=True)
                p = jnp.exp2(jnp.concatenate(tiles, axis=1) - m)
                l = jnp.sum(p, axis=-1, keepdims=True)
                r = pl.reciprocal(l, approx=True)
                r = r * (2.0 - l * r)
                ps.append(p * r)
            pf = jnp.concatenate(ps, axis=0)
            return [pf[:, k * 512:(k + 1) * 512].astype(bf16) for k in range(2)]

        def pv(u, p):
            br, j = divmod(u, GB)
            for n in range(2):
                o = None
                for k in range(2):
                    part = jnp.dot(
                        p[k], kvbuf[slot, 2 * br + 1, j, k * 512:(k + 1) * 512, n * 128:(n + 1) * 128],
                        preferred_element_type=f32)
                    stream.append((part, R2))
                    o = part if o is None else o + part
                ob = o.astype(bf16)
                obufs[br][j * SQ:(j + 1) * SQ, n * 128:(n + 1) * 128] = ob[:SQ]
                obufs[br][j * SQ:(j + 1) * SQ, DH + n * 128:DH + (n + 1) * 128] = ob[SQ:]

        def fence():
            @pl.when(it < 0)
            def _():
                wo_copy(0, 1 - slot, 0).start()

        def o_proj(br, t):
            if (br, t) != (0, 0) and not (br == 1 and t >= MT - 2):
                fence()
            r = jax.lax.dot_general(wobuf[slot, br], obufs[br][t * 128:(t + 1) * 128, :], NT,
                                    preferred_element_type=f32)
            stream.append((r, D))
            old = acc[br * D:(br + 1) * D, t * 128:(t + 1) * 128]
            new = jnp.where(first, 0.0, old) + r
            acc[br * D:(br + 1) * D, t * 128:(t + 1) * 128] = new
            if not (br == 1 and t == MT - 1):
                stage_tile(br, t, g, new, last)

        stage_tile(1, MT - 1, jnp.maximum(it - 1, 0) >> 3, acc[D:2 * D, last_tile], it == HKV)

        pending = []
        for i, pos in enumerate(QPOS):
            if pos == -1:
                qb_proj(i)
        s_cur = qk(0)
        for u in range(NU):
            br, j = divmod(u, GB)
            if u + 1 < NU:
                s_nxt = qk(u + 1)
            if u == 0:
                @pl.when(it < NIT - 1)
                def _():
                    nit = jnp.minimum(it + 1, NIT - 1)
                    start_slot(1 - slot, nit >> 3, nit & 7)
            for i, pos in enumerate(QPOS):
                if pos == u:
                    qb_proj(i)
            if pending:
                o_proj(*pending.pop(0))
            pv(u, softmax(*s_cur))
            s_cur = s_nxt
            pending.append((br, j))
            if j == GB - 1:
                pending.append((br, GB))
        for t in pending:
            o_proj(*t)
        return carry

    jax.lax.fori_loop(0, NIT, body, 0)

    stage_tile(1, MT - 1, NG - 1, acc[D:2 * D, last_tile], None)
    wait_all(stage, S_OUT)


@jax.jit
def pallas_concat_heads__gqa_block_cached__gqa_block_cached__near_ridge_kernel(
    A_x: jax.Array,
    A_k_cache: jax.Array,
    A_v_cache: jax.Array,
    A_wq: jax.Array,
    A_wo: jax.Array,
    B_x: jax.Array,
    B_k_cache: jax.Array,
    B_v_cache: jax.Array,
    B_wq: jax.Array,
    B_wo: jax.Array,
):
    any_spec = pl.BlockSpec(memory_space=pl.ANY)
    scratch = [
        pltpu.VMEM((2, 4, GB, SK, DH), bf16),
        pltpu.VMEM((M, D), bf16),
        pltpu.VMEM((M, D), bf16),
        pltpu.VMEM((HKV, D, GW), bf16),
        pltpu.VMEM((HKV, D, GW), bf16),
        pltpu.VMEM((2, 2, D, GW), bf16),
        pltpu.VMEM((HKV, M, GW), bf16),
        pltpu.VMEM((GR, GW), bf16),
        pltpu.VMEM((GR, GW), bf16),
        pltpu.VMEM((GR, GW), bf16),
        pltpu.VMEM((2 * D, GR), f32),
        pltpu.VMEM((M, 2 * D), bf16),
        pltpu.SemaphoreType.DMA((NSEM,)),
    ]
    out = pl.pallas_call(
        _kernel,
        in_specs=[any_spec] * 10,
        out_specs=any_spec,
        out_shape=jax.ShapeDtypeStruct((M, 2 * D), bf16),
        scratch_shapes=scratch,
        compiler_params=pltpu.CompilerParams(
            vmem_limit_bytes=120 * 1024 * 1024,
            disable_bounds_checks=True,
            disable_semaphore_checks=True,
        ),
    )(A_x.reshape(M, D), A_k_cache, A_v_cache, A_wq, A_wo.T,
      B_x.reshape(M, D), B_k_cache, B_v_cache, B_wq, B_wo.T)
    return out.reshape(B, SQ, 2 * D)
```

```python
import math

import jax
import jax.numpy as jnp
import jax.experimental.pallas as pl
import jax.experimental.pallas.tpu as pltpu

B, SQ, D = 16, 144, 448
HQ, HKV, SK, DH = 16, 8, 1024, 256
REP = HQ // HKV
GW = REP * DH
SSCALE = (DH ** -0.5) * math.log2(math.e)
NT = (((1,), (1,)), ((), ()))
GB = 8
NG = B // GB
GR = GB * SQ
MT = GR // 128
NU = 2 * GB
NIT = NG * HKV
M = B * SQ
R2 = REP * SQ
CA = 384
CH = 8
MARGIN = 400
QB = 2
QPOS = (-1, -1, 0, 1)
XROWS = (128, 336, 688, 1152)
f32, bf16 = jnp.float32, jnp.bfloat16
S_WQ, S_WQB, S_KV, S_WO, S_OUT, S_XB, S_X = 0, 3, 4, 6, 8, 9, 10
NSEM = S_X + len(XROWS)


def _kernel(xa, ka, va, wqa, woa, xb, kb, vb, wqb, wob, out_hbm,
            kvbuf, xbuf_a, xbuf_b, wqbuf_a, wqbuf_b, wobuf, qbuf_a, qbuf_b, obuf_a, obuf_b,
            acc, stage, sems):
    kv_hbm = (ka, va, kb, vb)
    wo_hbm = (woa, wob)
    obufs = (obuf_a, obuf_b)
    last_tile = slice((MT - 1) * 128, MT * 128)

    def wait_all(buf, sem):
        pltpu.make_async_copy(buf, buf, sems.at[sem]).wait()

    def wo_copy(br, slot, h):
        col = h * GW if isinstance(h, int) else pl.multiple_of(h * GW, GW)
        return pltpu.make_async_copy(wo_hbm[br].at[:, pl.ds(col, GW)], wobuf.at[slot, br],
                                     sems.at[S_WO + slot])

    def start_slot(slot, g, h):
        for i in range(4):
            pltpu.make_async_copy(kv_hbm[i].at[pl.ds(g * GB, GB), h], kvbuf.at[slot, i],
                                  sems.at[S_KV + slot]).start()
        for br in range(2):
            wo_copy(br, slot, h).start()

    def wqa_copy(h):
        return pltpu.make_async_copy(wqa.at[:, pl.ds(h * GW, GW)], wqbuf_a.at[h],
                                     sems.at[S_WQ + (0 if h == 0 else 1 if h < 4 else 2)])

    xp = []
    r0 = 0
    for n in XROWS:
        xp.append((r0, n))
        r0 += n

    def xa_copy(i):
        r, n = xp[i]
        return pltpu.make_async_copy(xa.at[pl.ds(r, n)], xbuf_a.at[pl.ds(r, n)], sems.at[S_X + i])

    def out_copy(row, br):
        cols = pl.ds(0, CA) if br == 0 else pl.ds(CA, 2 * D - CA)
        return pltpu.make_async_copy(stage.at[pl.ds(row, 128), cols],
                                     out_hbm.at[pl.ds(row, 128), cols], sems.at[S_OUT])

    wqa_copy(0).start()
    for i in range(len(xp) - 1):
        xa_copy(i).start()
    for h in range(1, HKV):
        wqa_copy(h).start()
    xa_copy(len(xp) - 1).start()
    pltpu.make_async_copy(xb, xbuf_b, sems.at[S_XB]).start()
    for h in range(HKV):
        pltpu.make_async_copy(wqb.at[:, pl.ds(h * GW, GW)], wqbuf_b.at[h], sems.at[S_WQB]).start()
    start_slot(0, 0, 0)

    def qa_rows(h, r, n):
        q = jnp.dot(xbuf_a[pl.ds(r, n), :], wqbuf_a[h], preferred_element_type=f32)
        qbuf_a[h, pl.ds(r, n), :] = q.astype(bf16)

    acc[CA:2 * D, last_tile] = jnp.zeros((2 * D - CA, 128), f32)
    wqa_copy(0).wait()
    for i in range(len(xp) - 1):
        xa_copy(i).wait()
        qa_rows(0, *xp[i])
    wait_all(wqbuf_a.at[pl.ds(1, 3)], S_WQ + 1)

    def p1_body(i, carry):
        @pl.when(i == 1)
        def _():
            wait_all(wqbuf_a.at[pl.ds(4, HKV - 4)], S_WQ + 2)
            xa_copy(len(xp) - 1).wait()

        for k in range(1, 4):
            idx = 3 * i + k
            qa_rows(idx & 7, pl.multiple_of(GR * (idx >> 3), GR), GR)
        return carry

    jax.lax.fori_loop(0, 5, p1_body, 0)
    wait_all(xbuf_b, S_XB)
    wait_all(wqbuf_b, S_WQB)

    def stage_tile(br, t, g, val, cond):
        row = g * GR + t * 128
        if not isinstance(row, int):
            row = pl.multiple_of(row, 128)
        if br == 0:
            stage[pl.ds(row, 128), 0:CA] = val[0:CA].T.astype(bf16)
        else:
            full = jnp.concatenate([acc[CA:D, t * 128:(t + 1) * 128], val], axis=0)
            stage[pl.ds(row, 128), CA:2 * D] = full.T.astype(bf16)
        if cond is None:
            out_copy(row, br).start()
        else:
            @pl.when(cond)
            def _():
                out_copy(row, br).start()

    def body(it, carry):
        g = it >> 3
        h = it & 7
        slot = it & 1
        wait_all(kvbuf.at[slot], S_KV + slot)
        wait_all(wobuf.at[slot], S_WO + slot)
        first = h == 0
        last = h == HKV - 1
        always = it >= 0
        stream = []

        def qb_proj(i):
            n = QB * SQ
            row = pl.multiple_of(g * GR + i * n, 16)
            x = xbuf_b[pl.ds(row, n), :]
            for c in range(4):
                q = jnp.dot(x, wqbuf_b[h, :, c * 128:(c + 1) * 128], preferred_element_type=f32)
                stream.append((q, n))
                qbuf_b[i * n:(i + 1) * n, c * 128:(c + 1) * 128] = q.astype(bf16)

        def qk(u):
            br, j = divmod(u, GB)
            if br == 0:
                rows = pl.ds(pl.multiple_of((g * GB + j) * SQ, 16), SQ)
                q2 = jnp.concatenate([qbuf_a[h, rows, 0:DH], qbuf_a[h, rows, DH:2 * DH]], axis=0)
            else:
                rows = slice(j * SQ, (j + 1) * SQ)
                q2 = jnp.concatenate([qbuf_b[rows, 0:DH], qbuf_b[rows, DH:2 * DH]], axis=0)
            s4 = [jax.lax.dot_general(q2, kvbuf[slot, 2 * br, j, c * 256:(c + 1) * 256, :], NT,
                                      preferred_element_type=f32) for c in range(4)]
            stream.extend((x, R2) for x in s4)
            return [x.astype(bf16).astype(f32) * SSCALE for x in s4], len(stream)

        def tokens(start, n):
            win = stream[start:]
            total = sum(nr for _, nr in win) - MARGIN
            out = []
            for c in range(n):
                pos = c * total // n
                for val, nr in win:
                    if pos < nr:
                        break
                    pos -= nr
                r = min((pos // 8) * 8, nr - CH)
                out.append(val[r:r + CH, 0:128])
            return out

        def softmax(s4, start):
            nch = R2 // CH
            toks = tokens(start, nch)
            ps = []
            for c in range(nch):
                rows = slice(c * CH, (c + 1) * CH)
                tiles = [x[rows, k * 128:(k + 1) * 128] for x in s4 for k in range(2)]
                m = jnp.where(always, tiles[0], toks[c])
                for t in tiles[1:]:
                    m = jnp.maximum(m, t)
                m = jnp.max(m, axis=-1, keepdims=True)
                p = jnp.exp2(jnp.concatenate(tiles, axis=1) - m)
                l = jnp.sum(p, axis=-1, keepdims=True)
                r = pl.reciprocal(l, approx=True)
                r = r * (2.0 - l * r)
                ps.append(p * r)
            pf = jnp.concatenate(ps, axis=0)
            return [pf[:, k * 512:(k + 1) * 512].astype(bf16) for k in range(2)]

        def pv(u, p):
            br, j = divmod(u, GB)
            for n in range(2):
                o = None
                for k in range(2):
                    part = jnp.dot(
                        p[k], kvbuf[slot, 2 * br + 1, j, k * 512:(k + 1) * 512, n * 128:(n + 1) * 128],
                        preferred_element_type=f32)
                    stream.append((part, R2))
                    o = part if o is None else o + part
                ob = o.astype(bf16)
                obufs[br][j * SQ:(j + 1) * SQ, n * 128:(n + 1) * 128] = ob[:SQ]
                obufs[br][j * SQ:(j + 1) * SQ, DH + n * 128:DH + (n + 1) * 128] = ob[SQ:]

        def fence():
            @pl.when(it < 0)
            def _():
                wo_copy(0, 1 - slot, 0).start()

        def o_proj(br, t):
            if (br, t) != (0, 0) and not (br == 1 and t >= MT - 2):
                fence()
            r = jax.lax.dot_general(wobuf[slot, br], obufs[br][t * 128:(t + 1) * 128, :], NT,
                                    preferred_element_type=f32)
            stream.append((r, D))
            old = acc[br * D:(br + 1) * D, t * 128:(t + 1) * 128]
            new = jnp.where(first, 0.0, old) + r
            acc[br * D:(br + 1) * D, t * 128:(t + 1) * 128] = new
            if not (br == 1 and t == MT - 1):
                stage_tile(br, t, g, new, last)

        stage_tile(1, MT - 1, jnp.maximum(it - 1, 0) >> 3, acc[D:2 * D, last_tile], it == HKV)

        pending = []
        for i, pos in enumerate(QPOS):
            if pos == -1:
                qb_proj(i)
        s_cur = qk(0)
        for u in range(NU):
            br, j = divmod(u, GB)
            if u + 1 < NU:
                s_nxt = qk(u + 1)
            if u == 0:
                @pl.when(it < NIT - 1)
                def _():
                    nit = jnp.minimum(it + 1, NIT - 1)
                    start_slot(1 - slot, nit >> 3, nit & 7)
            for i, pos in enumerate(QPOS):
                if pos == u:
                    qb_proj(i)
            if pending:
                o_proj(*pending.pop(0))
            pv(u, softmax(*s_cur))
            s_cur = s_nxt
            pending.append((br, j))
            if j == GB - 1:
                pending.append((br, GB))
        for t in pending:
            o_proj(*t)
        return carry

    jax.lax.fori_loop(0, NIT, body, 0)

    stage_tile(1, MT - 1, NG - 1, acc[D:2 * D, last_tile], None)
    pltpu.make_async_copy(stage, out_hbm, sems.at[S_OUT]).wait()


@jax.jit
def pallas_concat_heads__gqa_block_cached__gqa_block_cached__near_ridge_kernel(
    A_x: jax.Array,
    A_k_cache: jax.Array,
    A_v_cache: jax.Array,
    A_wq: jax.Array,
    A_wo: jax.Array,
    B_x: jax.Array,
    B_k_cache: jax.Array,
    B_v_cache: jax.Array,
    B_wq: jax.Array,
    B_wo: jax.Array,
):
    any_spec = pl.BlockSpec(memory_space=pl.ANY)
    scratch = [
        pltpu.VMEM((2, 4, GB, SK, DH), bf16),
        pltpu.VMEM((M, D), bf16),
        pltpu.VMEM((M, D), bf16),
        pltpu.VMEM((HKV, D, GW), bf16),
        pltpu.VMEM((HKV, D, GW), bf16),
        pltpu.VMEM((2, 2, D, GW), bf16),
        pltpu.VMEM((HKV, M, GW), bf16),
        pltpu.VMEM((GR, GW), bf16),
        pltpu.VMEM((GR, GW), bf16),
        pltpu.VMEM((GR, GW), bf16),
        pltpu.VMEM((2 * D, GR), f32),
        pltpu.VMEM((M, 2 * D), bf16),
        pltpu.SemaphoreType.DMA((NSEM,)),
    ]
    out = pl.pallas_call(
        _kernel,
        in_specs=[any_spec] * 10,
        out_specs=any_spec,
        out_shape=jax.ShapeDtypeStruct((M, 2 * D), bf16),
        scratch_shapes=scratch,
        compiler_params=pltpu.CompilerParams(
            vmem_limit_bytes=120 * 1024 * 1024,
            disable_bounds_checks=True,
            disable_semaphore_checks=True,
        ),
    )(A_x.reshape(M, D), A_k_cache, A_v_cache, A_wq, A_wo.T,
      B_x.reshape(M, D), B_k_cache, B_v_cache, B_wq, B_wo.T)
    return out.reshape(B, SQ, 2 * D)
```

```python
import math
import os

import jax
import jax.numpy as jnp
import jax.experimental.pallas as pl
import jax.experimental.pallas.tpu as pltpu

B, SQ, D = 16, 144, 448
HQ, HKV, SK, DH = 16, 8, 1024, 256
REP = HQ // HKV
GW = REP * DH
SSCALE = (DH ** -0.5) * math.log2(math.e)
NT = (((1,), (1,)), ((), ()))
GB = 8
NG = B // GB
GR = GB * SQ
MT = GR // 128
NU = 2 * GB
NIT = NG * HKV
M = B * SQ
R2 = REP * SQ
CA = 384
HD = D // 2
E = lambda k, d: int(os.environ.get(k, str(d)))
MARGIN = E('MARGIN', 500)
LAG = E('LAG', 950)
NBP = E('NBP', 32)
DLAG = E('DLAG', 160)
OPQ = E('OPQ', 1)
OPQE = E('OPQE', 1)
DPH = E('DPH', 10)
GA = E('GA', 4)
DGATE = E('DGATE', 1)
GT = E('GT', 0)
PMX = E('PMX', 1)
BLEAD = E('BLEAD', 300)
BMARGIN = E('BMARGIN', 200)
BSPAN = E('BSPAN', 2000)
QB = E('QB', 2)
OM = E('OM', 100)
OLEAD = E('OLEAD', 150)
OSPAN = E('OSPAN', 600)
FEN = E('FEN', 0)
OPOS = tuple(int(v) for v in os.environ.get('OPOS', '2,4,6,8,16,11,14,15,16,16').split(','))
QPOS = tuple(int(v) for v in os.environ.get('QPOS', '-1,0,10,12').split(','))
XROWS = (128, 336, 688, 1152)
f32, bf16, u32 = jnp.float32, jnp.bfloat16, jnp.uint32
S_WQ, S_WQB, S_KV, S_WO, S_OUT, S_XB, S_X = 0, 3, 4, 8, 10, 11, 12
NSEM = S_X + len(XROWS)
A11, A12, A22, S1, S2, S3, S4 = range(7)


def _cat(xs, axis):
    return xs[0] if len(xs) == 1 else jnp.concatenate(xs, axis=axis)


def _kernel(xa, ka, va, wqa, woa, xb, kb, vb, wqb, wob, out_hbm,
            kbuf, vbuf, xbuf_a, xbuf_b, wqbuf_a, wqbuf_b, wobuf, qbuf_a, qbuf_b, obuf_a, obuf_b,
            acc, stage, abuf0, abuf1, tbuf0, tbuf1, sbuf0, sbuf1, ebuf0, ebuf1, mbuf0, mbuf1, wsa, wsb, ot0, ot1, sems):
    kv_hbm = (ka, va, kb, vb)
    wo_hbm = (woa, wob)
    obufs = (obuf_a, obuf_b)
    abufs, tbufs = (abuf0, abuf1), (tbuf0, tbuf1)
    sbufs, ebufs, mbufs = (sbuf0, sbuf1), (ebuf0, ebuf1), (mbuf0, mbuf1)
    k32, v32, wo32, qa32, qb32 = (r.bitcast(u32) for r in (kbuf, vbuf, wobuf, qbuf_a, qbuf_b))
    o32 = tuple(r.bitcast(u32) for r in obufs)
    a32 = tuple(r.bitcast(u32) for r in abufs)
    t32 = tuple(r.bitcast(u32) for r in tbufs)
    wsbufs, otbufs = (wsa, wsb), (ot0, ot1)
    ws32 = tuple(r.bitcast(u32) for r in wsbufs)
    ot32 = tuple(r.bitcast(u32) for r in otbufs)
    tob = lambda x: pltpu.bitcast(x, bf16)
    last_tile = slice((MT - 1) * 128, MT * 128)

    def wait_all(buf, sem):
        pltpu.make_async_copy(buf, buf, sems.at[sem]).wait()

    def wo_copy(br, c, slot, h):
        col = h * GW + c * 128
        if not isinstance(col, int):
            col = pl.multiple_of(col, 128)
        return pltpu.make_async_copy(wo_hbm[br].at[:, pl.ds(col, 128)], wobuf.at[slot, br, c],
                                     sems.at[S_WO + slot])

    def start_kv(slot, i, j, g, h):
        for c in range(2):
            pltpu.make_async_copy(kv_hbm[i].at[g * GB + j, h, :, pl.ds(c * 128, 128)],
                                  (kbuf, vbuf)[i % 2].at[slot, i // 2, c, j],
                                  sems.at[S_KV + 2 * slot + i % 2]).start()

    def start_wo(slot, br, h):
        for c in range(4):
            wo_copy(br, c, slot, h).start()

    def wqa_copy(h):
        return pltpu.make_async_copy(wqa.at[:, pl.ds(h * GW, GW)], wqbuf_a.at[h],
                                     sems.at[S_WQ + (0 if h == 0 else 1 if h < 4 else 2)])

    xp = []
    r0 = 0
    for n in XROWS:
        xp.append((r0, n))
        r0 += n

    def xa_copy(i):
        r, n = xp[i]
        return pltpu.make_async_copy(xa.at[pl.ds(r, n)], xbuf_a.at[pl.ds(r, n)], sems.at[S_X + i])

    def out_copy(row, br):
        cols = pl.ds(0, CA) if br == 0 else pl.ds(CA, 2 * D - CA)
        return pltpu.make_async_copy(stage.at[pl.ds(row, 128), cols],
                                     out_hbm.at[pl.ds(row, 128), cols], sems.at[S_OUT])

    wqa_copy(0).start()
    for i in range(len(xp) - 1):
        xa_copy(i).start()
    for h in range(1, HKV):
        wqa_copy(h).start()
    xa_copy(len(xp) - 1).start()
    pltpu.make_async_copy(xb, xbuf_b, sems.at[S_XB]).start()
    for h in range(HKV):
        pltpu.make_async_copy(wqb.at[:, pl.ds(h * GW, GW)], wqbuf_b.at[h], sems.at[S_WQB]).start()
    for i0 in range(2):
        for i in range(4):
            for c in range(2):
                pltpu.make_async_copy(kv_hbm[i].at[pl.ds(0, GB), i0, :, pl.ds(c * 128, 128)],
                                      (kbuf, vbuf)[i % 2].at[i0, i // 2, c],
                                      sems.at[S_KV + 2 * i0 + i % 2]).start()
        for br in range(2):
            start_wo(i0, br, i0)

    def qa_rows(h, gq, r, n):
        row = gq * GR + r
        if not isinstance(row, int):
            row = pl.multiple_of(row, 16)
        q = jnp.dot(xbuf_a[pl.ds(row, n), :], wqbuf_a[h], preferred_element_type=f32)
        for c in range(4):
            qbuf_a[h, c, gq, r:r + n, :] = q[:, c * 128:(c + 1) * 128].astype(bf16)

    acc[CA:2 * D, last_tile] = jnp.zeros((2 * D - CA, 128), f32)
    wqa_copy(0).wait()
    for i in range(len(xp) - 1):
        xa_copy(i).wait()
        qa_rows(0, 0, *xp[i])
    wait_all(wqbuf_a.at[pl.ds(1, 3)], S_WQ + 1)

    def p1_body(i, carry):
        @pl.when(i == 1)
        def _():
            wait_all(wqbuf_a.at[pl.ds(4, HKV - 4)], S_WQ + 2)
            xa_copy(len(xp) - 1).wait()

        for k in range(1, 4):
            idx = 3 * i + k
            qa_rows(idx & 7, idx >> 3, 0, GR)
        return carry

    jax.lax.fori_loop(0, 5, p1_body, 0)
    wait_all(xbuf_b, S_XB)
    wait_all(wqbuf_b, S_WQB)

    def stage_tile(br, t, g, val, cond):
        row = g * GR + t * 128
        if not isinstance(row, int):
            row = pl.multiple_of(row, 128)
        if br == 0:
            stage[pl.ds(row, 128), 0:CA] = val[0:CA].T.astype(bf16)
        else:
            full = jnp.concatenate([acc[CA:D, t * 128:(t + 1) * 128], val], axis=0)
            stage[pl.ds(row, 128), CA:2 * D] = full.T.astype(bf16)
        if cond is None:
            out_copy(row, br).start()
        else:
            @pl.when(cond)
            def _():
                out_copy(row, br).start()

    plan = []
    for i, pos in enumerate(QPOS):
        if pos == -1:
            plan.append(("q", i))
    plan.append(("qk", 0))
    oops = [(k, (br, p)) for br in range(2) for k, p in [("o2", 0), ("o2", 1), ("o2", 2), ("o2", 3), ("o", MT - 1)]]
    for u in range(NU + 1):
        if u + 1 < NU:
            plan.append(("qk", u + 1))
        for i, pos in enumerate(QPOS):
            if pos == u:
                plan.append(("q", i))
        for op, pos in zip(oops, OPOS):
            if pos == u:
                plan.append(op)
        if u < NU:
            plan.append(("pv", u))
    assert plan[-1] == ("o", (1, MT - 1))
    last_wo = {br: [op for op in plan if op[0] in ("o", "o2") and op[1][0] == br][-1] for br in range(2)}
    dur = {"q": 4 * QB * SQ, "qk": 4 * R2, "o": D, "o2": 7 * HD // 2, "pv": 7 * SQ}
    tstart, tend = {}, {}
    tt = 0
    for op in plan:
        tstart[op] = tt
        tt += dur[op[0]]
        tend[op] = tt

    def body(it, carry):
        g = it >> 3
        h = it & 7
        slot = it & 1
        wait_all(kbuf.at[slot], S_KV + 2 * slot)
        wait_all(vbuf.at[slot], S_KV + 2 * slot + 1)
        wait_all(wobuf.at[slot], S_WO + slot)
        first = h == 0
        last = h == HKV - 1
        always = it >= 0
        zl = it >> 9
        st = {"now": 0}
        tasks = []
        gates = []

        def add_task(t, fn):
            tasks.append((t, len(tasks), fn))

        def add_gate(t, buf32):
            gates.append((t, buf32[zl, 0, 0:8, :]))

        def issue(ld32, nrows, ntiles, dot):
            t0 = st["now"]
            st["now"] = t0 + nrows
            if ntiles is None:
                return dot(ld32()), t0
            mine = [x for x in gates if x[0] < t0 + nrows]
            gates[:] = [x for x in gates if x[0] >= t0 + nrows]
            byrg = {}
            for t, mk in mine:
                byrg.setdefault(max(t - t0, 0) // 16, []).append(mk)
            parts, r = [], 0
            for rg in sorted(byrg):
                if rg * 16 > r:
                    parts.append(ld32(0, r, rg * 16))
                tile = ld32(0, rg * 16, rg * 16 + 16)
                for mk in byrg[rg]:
                    tile = jnp.where(always, tile, mk)
                parts.append(tile)
                r = rg * 16 + 16
            if r < nrows:
                parts.append(ld32(0, r, nrows))
            lhs = _cat([tob(_cat(parts, 0))] + [tob(ld32(c, 0, nrows)) for c in range(1, ntiles)], 1)
            return dot(lhs), t0

        def run_tasks(res, t0, nrows):
            while True:
                ready = sorted((x for x in tasks if x[0] < t0 + nrows), key=lambda x: x[:2])
                if not ready:
                    break
                x = ready[0]
                tasks.remove(x)
                r = min((max(x[0] - t0, 0) // 8) * 8, nrows - 8)
                x[2](res[r:r + 8, 0:128])

        def qb_proj(i):
            n = QB * SQ
            row = pl.multiple_of(g * GR + i * n, 16)
            x = xbuf_b[pl.ds(row, n), :]
            for c in range(4):
                q, t0 = issue(lambda: x, n, None, lambda x: jnp.dot(x, wqbuf_b[h, :, c * 128:(c + 1) * 128],
                                                                    preferred_element_type=f32))
                qbuf_b[c, i * n:(i + 1) * n, :] = q.astype(bf16)
                run_tasks(q, t0, n)

        def qk(u):
            br, j = divmod(u, GB)

            def ld1(c, a, b):
                if br == 0:
                    return qa32[h, c, g, (j * SQ + a) // 2:(j * SQ + b) // 2, :]
                return qb32[c, (j * SQ + a) // 2:(j * SQ + b) // 2, :]

            def ld(c, a, b):
                ps = []
                if a < SQ:
                    ps.append(ld1(c, a, min(b, SQ)))
                if b > SQ:
                    ps.append(ld1(2 + c, max(a, SQ) - SQ, b - SQ))
                return _cat(ps, 0)

            for c in range(4):
                kw = _cat([tob(k32[slot, br, d, j, c * 128:(c + 1) * 128, :]) for d in range(2)], 1)
                s, t0 = issue(ld, R2, 2, lambda x: jax.lax.dot_general(x, kw, NT, preferred_element_type=f32))
                sbufs[u % 2][0, :, c * 256:(c + 1) * 256] = s.astype(bf16)
                pm = jnp.maximum(s[:, :128], s[:, 128:])
                if PMX:
                    mbufs[u % 2][0, c] = pm
                    mrun = None
                else:
                    mrun = pm if c == 0 else jnp.maximum(mrun, pm)
                run_tasks(s, t0, R2)
            plan_unit(u, mrun)

        def plan_unit(u, mrun):
            br, j = divmod(u, GB)
            ab, tb, sb, eb = abufs[u % 2], tbufs[u % 2], sbufs[u % 2], ebufs[u % 2]
            t_lo = tend[("qk", u)]
            t_hi = tstart[("pv", u)] - MARGIN
            span = t_hi - t_lo
            zo = zl if OPQ else 0
            rs = {}

            def mke(c):
                def fn(tok):
                    rows = slice(c * 8, (c + 1) * 8)
                    if PMX:
                        mb = mbufs[u % 2]
                        mr = jnp.maximum(jnp.maximum(mb[zl, 0, rows, :], mb[zl, 1, rows, :]),
                                         jnp.maximum(mb[zl, 2, rows, :], mb[zl, 3, rows, :]))
                    else:
                        mr = mrun[rows]
                    m = jnp.max(mr, axis=-1, keepdims=True).astype(bf16).astype(f32)
                    m = jnp.where(always, jnp.broadcast_to(m, (8, 128)), tok)
                    sv = sb[zo, rows, :].astype(f32)
                    e = jnp.exp2((sv - jnp.concatenate([m] * 8, axis=1)) * SSCALE)
                    l = jnp.sum(e, axis=-1, keepdims=True)
                    eb[0, rows, :] = e.astype(bf16)
                    r = pl.reciprocal(l, approx=True)
                    rs[c] = r * (2.0 - l * r)
                return fn

            def mkd(gi, k, t):
                def fn(tok):
                    def put(op, v):
                        ab[0, op * 4 + k, gi * 16:(gi + 1) * 16, :] = v.astype(bf16)
                    blk = []
                    for hd in range(2):
                        rr = [jnp.broadcast_to(rs[hd * 18 + 2 * gi + z], (8, 128)) for z in range(2)]
                        if hd >= DGATE:
                            rr = [jnp.where(always, x, tok) for x in rr]
                        r = jnp.concatenate(rr, axis=0)
                        rows = slice(hd * SQ + gi * 16, hd * SQ + gi * 16 + 16)
                        for kh in range(2):
                            blk.append(eb[zl if OPQE else 0, rows, kh * 512 + k * 128:kh * 512 + (k + 1) * 128].astype(f32) * r)
                    a11, a12, a21, a22 = blk
                    s1 = a21 + a22
                    s2 = s1 - a11
                    put(A11, a11)
                    put(A12, a12)
                    put(A22, a22)
                    put(S1, s1)
                    put(S2, s2)
                    put(S3, a11 - a21)
                    put(S4, a12 - s2)
                    if GA and k % GA == GA - 1:
                        add_gate(t + LAG, a32[u % 2])
                return fn

            nd = 1
            while (nd - DPH / 100.0) * span / (38.0 + nd) < DLAG:
                nd += 1
            step = span / (38.0 + nd)
            i = 0
            for gi in range(9):
                for hd in range(2):
                    for half in range(2):
                        add_task(t_lo + int(i * step), mke(hd * 18 + gi * 2 + half))
                        i += 1
                for k in range(4):
                    t = t_lo + int((i - 1 + k + nd - DPH / 100.0) * step)
                    add_task(t, mkd(gi, k, t))

        def plan_bp(u):
            br, j = divmod(u, GB)
            tb = tbufs[u % 2]
            nr = 512 // NBP
            t_lo = tend[("pv", u - 2)] + BLEAD if u >= 2 else (0 if u == 0 else tstart[("qk", 0)])
            t_hi = min(tstart[("pv", u)] - BMARGIN, t_lo + BSPAN)
            span = t_hi - t_lo

            def mkb(bi, t):
                def fn(tok):
                    vb = lambda k, n: vbuf[slot, br, n, j,
                                            k * 512 + bi * nr:k * 512 + (bi + 1) * nr, :].astype(f32)
                    b11, b12, b21, b22 = vb(0, 0), vb(0, 1), vb(1, 0), vb(1, 1)
                    b12 = jnp.where(always, b12, jnp.concatenate([tok] * (nr // 8), axis=0))
                    t1 = b12 - b11
                    t2 = b22 - t1
                    for ti, v in enumerate((t1, t2, b22 - b12, t2 - b21)):
                        tb[0, ti, bi * nr:(bi + 1) * nr, :] = v.astype(bf16)
                    if GT:
                        add_gate(t + LAG, t32[u % 2])
                return fn

            for bi in range(NBP):
                t = t_lo + (2 * bi + 1) * span // (2 * NBP)
                add_task(t, mkb(bi, t))

        def pv(u):
            br, j = divmod(u, GB)
            vb = lambda k, n: tob(v32[slot, br, n, j, k * 256:(k + 1) * 256, :])
            tw = lambda ti: tob(t32[u % 2][0, ti])

            def mm(op, wfn):
                ld = lambda c, a, b: a32[u % 2][0, op * 4 + c, a // 2:b // 2, :]
                r, t0 = issue(ld, SQ, 4, lambda x: jnp.dot(x, wfn(), preferred_element_type=f32))
                run_tasks(r, t0, SQ)
                return r

            rows = slice(j * SQ, (j + 1) * SQ)
            p1 = mm(A11, lambda: vb(0, 0))
            p2 = mm(A12, lambda: vb(1, 0))
            obufs[br][0, rows, :] = (p1 + p2).astype(bf16)
            u2 = p1 + mm(S2, lambda: tw(1))
            u3 = u2 + mm(S3, lambda: tw(2))
            p5 = mm(S1, lambda: tw(0))
            u4 = u2 + p5
            obufs[br][3, rows, :] = (u3 + p5).astype(bf16)
            obufs[br][1, rows, :] = (u4 + mm(S4, lambda: vb(1, 1))).astype(bf16)
            obufs[br][2, rows, :] = (u3 - mm(A22, lambda: tw(3))).astype(bf16)

        def fence():
            @pl.when(it < 0)
            def _():
                wo_copy(0, 0, 1 - slot, 0).start()

        def finish_tile(br, t, r):
            old = acc[br * D:(br + 1) * D, t * 128:(t + 1) * 128]
            new = jnp.where(first, 0.0, old) + r
            acc[br * D:(br + 1) * D, t * 128:(t + 1) * 128] = new
            if not (br == 1 and t == MT - 1):
                stage_tile(br, t, g, new, last)

        def o_proj(br, t):
            if FEN:
                fence()
            ld = lambda c, a, b: wo32[slot, br, c, a // 2:b // 2, :]
            ow = _cat([tob(o32[br][c, t * 64:(t + 1) * 64, :]) for c in range(4)], 1)
            r, t0 = issue(ld, D, 4, lambda x: jax.lax.dot_general(x, ow, NT, preferred_element_type=f32))
            finish_tile(br, t, r)
            run_tasks(r, t0, D)

        def spread(t_lo, t_hi, fns):
            for i, fn in enumerate(fns):
                add_task(t_lo + (2 * i + 1) * (t_hi - t_lo) // (2 * len(fns)), fn)

        def plan_ws(br):
            def mk(gi, c):
                def fn(tok):
                    w = lambda i, k: wobuf[slot, br, 2 * k + c, i * HD + gi * 16:i * HD + (gi + 1) * 16, :].astype(f32)
                    a11, a12, a21, a22 = w(0, 0), w(0, 1), w(1, 0), w(1, 1)
                    a21 = jnp.where(always, a21, jnp.concatenate([tok, tok], axis=0))
                    s1 = a21 + a22
                    s2 = s1 - a11
                    for i, v in enumerate((s1, s2, a11 - a21, a12 - s2)):
                        wsbufs[br][2 * i + c, gi * 16:(gi + 1) * 16, :] = v.astype(bf16)
                return fn
            t_lo = br * 1150
            spread(t_lo, t_lo + 1150, [mk(gi, c) for gi in range(HD // 16) for c in range(2)])

        def plan_ot(br, p):
            par = (br * 4 + p) % 2

            def mk(gi, c):
                def fn(tok):
                    o = lambda k, n: obufs[br][2 * k + c, (2 * p + n) * 128 + gi * 16:(2 * p + n) * 128 + (gi + 1) * 16,
                                               :].astype(f32)
                    b11, b12, b21, b22 = o(0, 0), o(0, 1), o(1, 0), o(1, 1)
                    b12 = jnp.where(always, b12, jnp.concatenate([tok, tok], axis=0))
                    t1 = b12 - b11
                    t2 = b22 - t1
                    for i, v in enumerate((t1, t2, b22 - b12, t2 - b21)):
                        otbufs[par][2 * i + c, gi * 16:(gi + 1) * 16, :] = v.astype(bf16)
                return fn
            t_hi = tstart[("o2", (br, p))] - OM
            t_lo = tend[("pv", br * GB + 2 * p + 1)] + OLEAD
            idx = br * 4 + p
            if idx >= 2:
                t_lo = max(t_lo, tend[("o2", divmod(idx - 2, 4))])
            t_lo = max(t_lo, t_hi - OSPAN)
            assert t_lo < t_hi, (br, p, t_lo, t_hi)
            spread(t_lo, t_hi, [mk(gi, c) for gi in range(8) for c in range(2)])

        def o_pair(br, p):
            if FEN:
                fence()
            par = (br * 4 + p) % 2
            wa = lambda i, k: (lambda c, a, b: wo32[slot, br, 2 * k + c, (i * HD + a) // 2:(i * HD + b) // 2, :])
            ws = lambda i: (lambda c, a, b: ws32[br][2 * i + c, a // 2:b // 2, :])
            ob = lambda k, n: _cat([tob(o32[br][2 * k + c, (2 * p + n) * 64:(2 * p + n + 1) * 64, :])
                                    for c in range(2)], 1)
            ot = lambda i: _cat([tob(ot32[par][2 * i + c]) for c in range(2)], 1)
            dot = lambda x, w: jax.lax.dot_general(x, w, NT, preferred_element_type=f32)

            def two(ld1, w1, ld2, w2, n):
                r1 = dot(_cat([tob(ld1(c, 0, n)) for c in range(2)], 1), w1)
                r2, t0 = issue(ld2, n, 2, lambda x: dot(x, w2))
                run_tasks(r2, t0, n)
                return r1, r2

            p1, p2 = two(wa(0, 0), ob(0, 0), wa(0, 1), ob(1, 0), HD)
            c11 = p1 + p2
            p6, p7 = two(ws(1), ot(1), ws(2), ot(2), HD)
            u2 = p1 + p6
            u3 = u2 + p7
            p5, p3 = two(ws(0), ot(0), ws(3), ob(1, 1), HD)
            finish_tile(br, 2 * p + 1, jnp.concatenate([u2 + p5 + p3, u3 + p5], axis=0))
            l22 = wa(1, 1)
            p4a, p4b = two(l22, ot(3), lambda c, a, b: l22(c, HD // 2 + a, HD // 2 + b), ot(3), HD // 2)
            finish_tile(br, 2 * p, jnp.concatenate([c11, u3 - jnp.concatenate([p4a, p4b], axis=0)], axis=0))

        stage_tile(1, MT - 1, jnp.maximum(it - 1, 0) >> 3, acc[D:2 * D, last_tile], it == HKV)

        for u in range(NU):
            plan_bp(u)
        for br in range(2):
            plan_ws(br)
            for p in range(4):
                plan_ot(br, p)
        nit = jnp.minimum(it + 2, NIT - 1)
        more = it < NIT - 2
        for kind, arg in plan:
            assert st["now"] == tstart[(kind, arg)]
            if kind == "q":
                qb_proj(arg)
            elif kind == "qk":
                qk(arg)
                pl.when(more)(lambda: start_kv(slot, 2 * (arg // GB), arg % GB, nit >> 3, nit & 7))
            elif kind in ("o", "o2"):
                (o_proj if kind == "o" else o_pair)(*arg)
            elif kind == "pv":
                pv(arg)
                pl.when(more)(lambda: start_kv(slot, 2 * (arg // GB) + 1, arg % GB, nit >> 3, nit & 7))
        assert not tasks

        @pl.when(more)
        def _():
            for br in range(2):
                start_wo(slot, br, nit & 7)
        return carry

    jax.lax.fori_loop(0, NIT, body, 0)

    stage_tile(1, MT - 1, NG - 1, acc[D:2 * D, last_tile], None)
    pltpu.make_async_copy(stage, out_hbm, sems.at[S_OUT]).wait()


@jax.jit
def pallas_concat_heads__gqa_block_cached__gqa_block_cached__near_ridge_kernel(
    A_x, A_k_cache, A_v_cache, A_wq, A_wo, B_x, B_k_cache, B_v_cache, B_wq, B_wo,
):
    any_spec = pl.BlockSpec(memory_space=pl.ANY)
    scratch = [
        pltpu.VMEM((2, 2, 2, GB, SK, 128), bf16),
        pltpu.VMEM((2, 2, 2, GB, SK, 128), bf16),
        pltpu.VMEM((M, D), bf16),
        pltpu.VMEM((M, D), bf16),
        pltpu.VMEM((HKV, D, GW), bf16),
        pltpu.VMEM((HKV, D, GW), bf16),
        pltpu.VMEM((2, 2, 4, D, 128), bf16),
        pltpu.VMEM((HKV, 4, NG, GR, 128), bf16),
        pltpu.VMEM((4, GR, 128), bf16),
        pltpu.VMEM((4, GR, 128), bf16),
        pltpu.VMEM((4, GR, 128), bf16),
        pltpu.VMEM((2 * D, GR), f32),
        pltpu.VMEM((M, 2 * D), bf16),
        pltpu.VMEM((2, 28, SQ, 128), bf16),
        pltpu.VMEM((2, 28, SQ, 128), bf16),
        pltpu.VMEM((2, 4, 512, 128), bf16),
        pltpu.VMEM((2, 4, 512, 128), bf16),
        pltpu.VMEM((2, R2, SK), bf16),
        pltpu.VMEM((2, R2, SK), bf16),
        pltpu.VMEM((2, R2, SK), bf16),
        pltpu.VMEM((2, R2, SK), bf16),
        pltpu.VMEM((2, 4, R2, 128), f32),
        pltpu.VMEM((2, 4, R2, 128), f32),
        pltpu.VMEM((8, HD, 128), bf16),
        pltpu.VMEM((8, HD, 128), bf16),
        pltpu.VMEM((8, 128, 128), bf16),
        pltpu.VMEM((8, 128, 128), bf16),
        pltpu.SemaphoreType.DMA((NSEM,)),
    ]
    out = pl.pallas_call(
        _kernel,
        in_specs=[any_spec] * 10,
        out_specs=any_spec,
        out_shape=jax.ShapeDtypeStruct((M, 2 * D), bf16),
        scratch_shapes=scratch,
        compiler_params=pltpu.CompilerParams(
            vmem_limit_bytes=120 * 1024 * 1024,
            disable_bounds_checks=True,
            disable_semaphore_checks=True,
        ),
    )(A_x.reshape(M, D), A_k_cache, A_v_cache, A_wq, A_wo.T,
      B_x.reshape(M, D), B_k_cache, B_v_cache, B_wq, B_wo.T)
    return out.reshape(B, SQ, 2 * D)
```

```python
import math

import jax
import jax.numpy as jnp
import jax.experimental.pallas as pl
import jax.experimental.pallas.tpu as pltpu

B, SQ, D = 16, 144, 448
HQ, HKV, SK, DH = 16, 8, 1024, 256
REP = HQ // HKV
GW = REP * DH
SSCALE = (DH ** -0.5) * math.log2(math.e)
NT = (((1,), (1,)), ((), ()))
GB = 8
NG = B // GB
GR = GB * SQ
MT = GR // 128
NU = 2 * GB
NIT = NG * HKV
M = B * SQ
R2 = REP * SQ
CA = 384
HD = D // 2
QB = 2
QPOS = (-1, 0, 10, 12)
OPOS = (2, 4, 6, 8, 16, 11, 14, 15, 16, 16)
MARGIN, LAG, DLAG, DPH, MINGAP = 500, 950, 160, 0.1, 12
BLEAD, BMARGIN, BSPAN = 300, 200, 2000
OM, OLEAD, OSPAN = 100, 150, 600
XROWS = (128, 336, 688, 1152)
f32, bf16, u32 = jnp.float32, jnp.bfloat16, jnp.uint32
S_WQ, S_WQB, S_KV, S_WO, S_OUT, S_XB, S_X = 0, 3, 4, 8, 10, 11, 12
NSEM = S_X + len(XROWS)
A11, A12, A22, S1, S2, S3, S4 = range(7)


def _cat(xs, axis):
    return xs[0] if len(xs) == 1 else jnp.concatenate(xs, axis=axis)


def _wide(tiles):
    return _cat([pltpu.bitcast(t, bf16) for t in tiles], 1)


def _lhs_sums(a11, a12, a21, a22):
    s1 = a21 + a22
    s2 = s1 - a11
    return s1, s2, a11 - a21, a12 - s2


def _rhs_sums(b11, b12, b21, b22):
    t1 = b12 - b11
    t2 = b22 - t1
    return t1, t2, b22 - b12, t2 - b21


def _kernel(xa, ka, va, wqa, woa, xb, kb, vb, wqb, wob, out_hbm,
            kbuf, vbuf, xbuf_a, xbuf_b, wqbuf_a, wqbuf_b, wobuf, qbuf_a, qbuf_b, obuf_a, obuf_b,
            acc, stage, abuf0, abuf1, tbuf0, tbuf1, sbuf0, sbuf1, ebuf0, ebuf1, mbuf0, mbuf1,
            wsa, wsb, ot0, ot1, sems):
    kv_hbm = (ka, va, kb, vb)
    wo_hbm = (woa, wob)
    obufs, abufs, tbufs = (obuf_a, obuf_b), (abuf0, abuf1), (tbuf0, tbuf1)
    sbufs, ebufs, mbufs = (sbuf0, sbuf1), (ebuf0, ebuf1), (mbuf0, mbuf1)
    wsbufs, otbufs = (wsa, wsb), (ot0, ot1)
    k32, v32, wo32, qa32, qb32 = (r.bitcast(u32) for r in (kbuf, vbuf, wobuf, qbuf_a, qbuf_b))
    o32, a32, t32, ws32, ot32 = (tuple(r.bitcast(u32) for r in rs)
                                 for rs in (obufs, abufs, tbufs, wsbufs, otbufs))
    last_tile = slice((MT - 1) * 128, MT * 128)

    def wait_all(buf, sem):
        pltpu.make_async_copy(buf, buf, sems.at[sem]).wait()

    def start_kv(slot, i, j, g, h):
        for c in range(2):
            pltpu.make_async_copy(kv_hbm[i].at[g * GB + j, h, :, pl.ds(c * 128, 128)],
                                  (kbuf, vbuf)[i % 2].at[slot, i // 2, c, j],
                                  sems.at[S_KV + 2 * slot + i % 2]).start()

    def start_wo(slot, h):
        for br in range(2):
            for c in range(4):
                col = h * GW + c * 128
                if not isinstance(col, int):
                    col = pl.multiple_of(col, 128)
                pltpu.make_async_copy(wo_hbm[br].at[:, pl.ds(col, 128)], wobuf.at[slot, br, c],
                                      sems.at[S_WO + slot]).start()

    def wqa_copy(h):
        return pltpu.make_async_copy(wqa.at[:, pl.ds(h * GW, GW)], wqbuf_a.at[h],
                                     sems.at[S_WQ + (0 if h == 0 else 1 if h < 4 else 2)])

    xp = []
    r0 = 0
    for n in XROWS:
        xp.append((r0, n))
        r0 += n

    def xa_copy(i):
        r, n = xp[i]
        return pltpu.make_async_copy(xa.at[pl.ds(r, n)], xbuf_a.at[pl.ds(r, n)], sems.at[S_X + i])

    def out_copy(row, br):
        cols = pl.ds(0, CA) if br == 0 else pl.ds(CA, 2 * D - CA)
        return pltpu.make_async_copy(stage.at[pl.ds(row, 128), cols],
                                     out_hbm.at[pl.ds(row, 128), cols], sems.at[S_OUT])

    wqa_copy(0).start()
    for i in range(len(xp) - 1):
        xa_copy(i).start()
    for h in range(1, HKV):
        wqa_copy(h).start()
    xa_copy(len(xp) - 1).start()
    pltpu.make_async_copy(xb, xbuf_b, sems.at[S_XB]).start()
    for h in range(HKV):
        pltpu.make_async_copy(wqb.at[:, pl.ds(h * GW, GW)], wqbuf_b.at[h], sems.at[S_WQB]).start()
    for i0 in range(2):
        for i in range(4):
            for c in range(2):
                pltpu.make_async_copy(kv_hbm[i].at[pl.ds(0, GB), i0, :, pl.ds(c * 128, 128)],
                                      (kbuf, vbuf)[i % 2].at[i0, i // 2, c],
                                      sems.at[S_KV + 2 * i0 + i % 2]).start()
        start_wo(i0, i0)

    def qa_rows(h, gq, r, n):
        row = gq * GR + r
        if not isinstance(row, int):
            row = pl.multiple_of(row, 16)
        q = jnp.dot(xbuf_a[pl.ds(row, n), :], wqbuf_a[h], preferred_element_type=f32)
        for c in range(4):
            qbuf_a[h, c, gq, r:r + n, :] = q[:, c * 128:(c + 1) * 128].astype(bf16)

    acc[CA:2 * D, last_tile] = jnp.zeros((2 * D - CA, 128), f32)
    wqa_copy(0).wait()
    for i in range(len(xp) - 1):
        xa_copy(i).wait()
        qa_rows(0, 0, *xp[i])
    wait_all(wqbuf_a.at[pl.ds(1, 3)], S_WQ + 1)

    def p1_body(i, carry):
        @pl.when(i == 1)
        def _():
            wait_all(wqbuf_a.at[pl.ds(4, HKV - 4)], S_WQ + 2)
            xa_copy(len(xp) - 1).wait()

        for k in range(1, 4):
            idx = 3 * i + k
            qa_rows(idx & 7, idx >> 3, 0, GR)
        return carry

    jax.lax.fori_loop(0, 5, p1_body, 0)
    wait_all(xbuf_b, S_XB)
    wait_all(wqbuf_b, S_WQB)

    def stage_tile(br, t, g, val, cond):
        row = g * GR + t * 128
        if not isinstance(row, int):
            row = pl.multiple_of(row, 128)
        if br == 0:
            stage[pl.ds(row, 128), 0:CA] = val[0:CA].T.astype(bf16)
        else:
            full = jnp.concatenate([acc[CA:D, t * 128:(t + 1) * 128], val], axis=0)
            stage[pl.ds(row, 128), CA:2 * D] = full.T.astype(bf16)
        if cond is None:
            out_copy(row, br).start()
        else:
            @pl.when(cond)
            def _():
                out_copy(row, br).start()

    plan = [("q", i) for i, pos in enumerate(QPOS) if pos == -1] + [("qk", 0)]
    oops = [(k, (br, p)) for br in range(2)
            for k, p in [("o2", 0), ("o2", 1), ("o2", 2), ("o2", 3), ("o", MT - 1)]]
    for u in range(NU + 1):
        if u + 1 < NU:
            plan.append(("qk", u + 1))
        plan += [("q", i) for i, pos in enumerate(QPOS) if pos == u]
        plan += [op for op, pos in zip(oops, OPOS) if pos == u]
        if u < NU:
            plan.append(("pv", u))
    assert plan[-1] == ("o", (1, MT - 1))
    dur = {"q": 4 * QB * SQ, "qk": 4 * R2, "o": D, "o2": 7 * HD // 2, "pv": 7 * SQ}
    tstart, tend = {}, {}
    tt = 0
    for op in plan:
        tstart[op] = tt
        tt += dur[op[0]]
        tend[op] = tt

    for i in range(len(QPOS)):
        assert tend[("q", i)] <= tstart[("qk", GB + QB * i)]

    def body(it, carry):
        g = it >> 3
        h = it & 7
        slot = it & 1
        wait_all(kbuf.at[slot], S_KV + 2 * slot)
        wait_all(vbuf.at[slot], S_KV + 2 * slot + 1)
        wait_all(wobuf.at[slot], S_WO + slot)
        first = h == 0
        last = h == HKV - 1
        always = it >= 0
        zl = it >> 9
        nit = jnp.minimum(it + 2, NIT - 1)
        more = it < NIT - 2
        st = {"now": 0, "free": 0, "seq": 0}
        tasks = []
        gates = []

        def add_task(key, t, fn):
            st["seq"] += 1
            tasks.append((t, st["seq"], fn, key))

        def done(*keys):
            assert not [x for x in tasks if x[3] in keys], keys

        def spread(key, t_lo, t_hi, fns):
            assert t_lo < t_hi
            for i, fn in enumerate(fns):
                add_task(key, t_lo + (2 * i + 1) * (t_hi - t_lo) // (2 * len(fns)), fn)

        def after(x, tok):
            return jnp.where(always, x, _cat([tok] * (x.shape[0] // 8), 0))

        def gated(tiles, nrows):
            t0 = st["now"]
            mine = [x for x in gates if x[0] < t0 + nrows]
            gates[:] = [x for x in gates if x[0] >= t0 + nrows]
            if mine:
                parts = [tiles[0][r * 8:(r + 1) * 8] for r in range(nrows // 16)]
                for t, mk in mine:
                    r = max(t - t0, 0) // 16
                    parts[r] = jnp.where(always, parts[r], mk)
                tiles = [_cat(parts, 0)] + list(tiles[1:])
            return _wide(tiles)

        def advance(res, nrows):
            t0 = st["now"]
            st["now"] = t0 + nrows
            tasks.sort(key=lambda x: x[:2])
            while tasks:
                t = max(tasks[0][0], st["free"], t0)
                if t >= t0 + nrows:
                    break
                fn = tasks.pop(0)[2]
                st["free"] = t + MINGAP
                r = ((t - t0) // 8) * 8
                fn(res[r:r + 8, 0:128])

        def qb_proj(i):
            n = QB * SQ
            x = xbuf_b[pl.ds(pl.multiple_of(g * GR + i * n, 16), n), :]
            for c in range(4):
                q = jnp.dot(x, wqbuf_b[h, :, c * 128:(c + 1) * 128], preferred_element_type=f32)
                qbuf_b[c, i * n:(i + 1) * n, :] = q.astype(bf16)
                advance(q, n)

        def qk(u):
            br, j = divmod(u, GB)
            rows = slice(j * SQ // 2, (j + 1) * SQ // 2)
            for c in range(4):
                q = qa32[h, :, g, rows, :] if br == 0 else qb32[:, rows, :]
                lhs = gated([_cat([q[d], q[2 + d]], 0) for d in range(2)], R2)
                kw = k32[slot, br, :, j, c * 128:(c + 1) * 128, :]
                s = jax.lax.dot_general(lhs, _wide([kw[0], kw[1]]), NT, preferred_element_type=f32)
                sbufs[u % 2][0, :, c * 256:(c + 1) * 256] = s.astype(bf16)
                mbufs[u % 2][0, c] = jnp.maximum(s[:, :128], s[:, 128:])
                advance(s, R2)
            plan_softmax(u)

        def plan_softmax(u):
            ab, sb, eb, mb = abufs[u % 2], sbufs[u % 2], ebufs[u % 2], mbufs[u % 2]
            t_lo = tend[("qk", u)]
            span = tstart[("pv", u)] - MARGIN - t_lo
            rs = {}

            def mke(hd, c):
                def fn(tok):
                    rows = slice(hd * SQ + c * 8, hd * SQ + (c + 1) * 8)
                    pm = mb[zl, :, rows, :]
                    m = jnp.maximum(jnp.maximum(pm[0], pm[1]), jnp.maximum(pm[2], pm[3]))
                    m = jnp.max(m, axis=-1, keepdims=True).astype(bf16).astype(f32)
                    m = after(jnp.broadcast_to(m, (8, 128)), tok)
                    e = jnp.exp2((sb[zl, rows, :].astype(f32) - _cat([m] * 8, 1)) * SSCALE)
                    l = jnp.sum(e, axis=-1, keepdims=True)
                    eb[0, hd, c * 8:(c + 1) * 8, :] = e.astype(bf16)
                    r = pl.reciprocal(l, approx=True)
                    rs[hd, c] = jnp.broadcast_to(r * (2.0 - l * r), (8, 128))
                return fn

            def mkd(gi, k, t):
                def fn(tok):
                    e = eb[zl, :, gi * 16:(gi + 1) * 16, k * 256:(k + 1) * 256].astype(f32)
                    r0 = _cat([rs[0, 2 * gi], rs[0, 2 * gi + 1]], 0)
                    r1 = after(_cat([rs[1, 2 * gi], rs[1, 2 * gi + 1]], 0), tok)
                    a11, a12 = e[0, :, :128] * r0, e[0, :, 128:] * r0
                    a21, a22 = e[1, :, :128] * r1, e[1, :, 128:] * r1
                    ab[0, k, gi] = _cat([a11, a12, a22, *_lhs_sums(a11, a12, a21, a22)], 0).astype(bf16)
                    if k == 3:
                        gates.append((t + LAG, a32[u % 2][zl, 0, 0, 0:8, :]))
                return fn

            nd = 1
            while (nd - DPH) * span / (38.0 + nd) < DLAG:
                nd += 1
            step = span / (38.0 + nd)
            i = 0
            for gi in range(9):
                for hd in range(2):
                    for half in range(2):
                        add_task(("p", u), t_lo + int(i * step), mke(hd, gi * 2 + half))
                        i += 1
                for k in range(4):
                    t = t_lo + int((i - 1 + k + nd - DPH) * step)
                    add_task(("p", u), t, mkd(gi, k, t))

        def plan_vsums(u):
            br, j = divmod(u, GB)

            def mk(bi):
                def fn(tok):
                    r = (bi // 8) * 256 + (bi % 8) * 16
                    v1 = vbuf[slot, br, :, j, r:r + 16, :].astype(f32)
                    v2 = vbuf[slot, br, :, j, r + 128:r + 144, :].astype(f32)
                    tbufs[u % 2][bi] = _cat(list(_rhs_sums(v1[0], after(v1[1], tok), v2[0], v2[1])), 0).astype(bf16)
                return fn
            t_lo = tend[("pv", u - 2)] + BLEAD if u >= 2 else (0 if u == 0 else tstart[("qk", 0)])
            spread(("v", u), t_lo, min(tstart[("pv", u)] - BMARGIN, t_lo + BSPAN), [mk(bi) for bi in range(32)])

        def refill(kv, u):
            pl.when(more)(lambda: start_kv(slot, 2 * (u // GB) + kv, u % GB, nit >> 3, nit & 7))

        def pv(u):
            br, j = divmod(u, GB)

            def vraw(kh, n):
                v = v32[slot, br, n, j]
                return pltpu.bitcast(_cat([v[k * 128 + kh * 64:k * 128 + (kh + 1) * 64] for k in range(4)], 0), bf16)

            def vsum(i):
                return pltpu.bitcast(t32[u % 2][:, i * 8:(i + 1) * 8, :].reshape(256, 128), bf16)

            def mm(op, w):
                a = a32[u % 2][0, :, :, op * 8:(op + 1) * 8, :]
                r = jnp.dot(gated([a[k].reshape(SQ // 2, 128) for k in range(4)], SQ), w,
                            preferred_element_type=f32)
                advance(r, SQ)
                return r

            rows = slice(j * SQ, (j + 1) * SQ)
            done(("p", u), ("v", u))
            p1 = mm(A11, vraw(0, 0))
            p2 = mm(A12, vraw(1, 0))
            obufs[br][0, rows, :] = (p1 + p2).astype(bf16)
            u2 = p1 + mm(S2, vsum(1))
            u3 = u2 + mm(S3, vsum(2))
            p5 = mm(S1, vsum(0))
            u4 = u2 + p5
            obufs[br][3, rows, :] = (u3 + p5).astype(bf16)
            if u == NU - 1:
                refill(1, u - 1)
            obufs[br][1, rows, :] = (u4 + mm(S4, vraw(1, 1))).astype(bf16)
            obufs[br][2, rows, :] = (u3 - mm(A22, vsum(3))).astype(bf16)

        def finish_tile(br, t, r):
            old = acc[br * D:(br + 1) * D, t * 128:(t + 1) * 128]
            new = jnp.where(first, 0.0, old) + r
            acc[br * D:(br + 1) * D, t * 128:(t + 1) * 128] = new
            if not (br == 1 and t == MT - 1):
                stage_tile(br, t, g, new, last)

        def o_single(br, t):
            w = wo32[slot, br]
            o = o32[br][:, t * 64:(t + 1) * 64, :]
            r = jax.lax.dot_general(gated([w[c] for c in range(4)], D), _wide([o[c] for c in range(4)]), NT,
                                    preferred_element_type=f32)
            finish_tile(br, t, r)
            advance(r, D)

        def plan_wsums(br):
            def mk(gi, c):
                def fn(tok):
                    w1 = wobuf[slot, br, :, gi * 16:(gi + 1) * 16, :].astype(f32)
                    w2 = wobuf[slot, br, :, HD + gi * 16:HD + (gi + 1) * 16, :].astype(f32)
                    wsbufs[br][c, gi] = _cat(list(_lhs_sums(w1[c], w1[2 + c], after(w2[c], tok), w2[2 + c])),
                                             0).astype(bf16)
                return fn
            spread(("w", br), br * 1150, (br + 1) * 1150, [mk(gi, c) for gi in range(HD // 16) for c in range(2)])

        def plan_osums(br, p):
            idx = br * 4 + p

            def mk(gi, c):
                def fn(tok):
                    r = 2 * p * 128 + gi * 16
                    o1 = obufs[br][:, r:r + 16, :].astype(f32)
                    o2 = obufs[br][:, r + 128:r + 144, :].astype(f32)
                    otbufs[idx % 2][c, gi] = _cat(list(_rhs_sums(o1[c], after(o2[c], tok), o1[2 + c], o2[2 + c])),
                                                  0).astype(bf16)
                return fn
            t_hi = tstart[("o2", (br, p))] - OM
            t_lo = max(tend[("pv", br * GB + 2 * p + 1)] + OLEAD, t_hi - OSPAN)
            if idx >= 2:
                t_lo = max(t_lo, tend[("o2", divmod(idx - 2, 4))])
            spread(("o", idx), t_lo, t_hi, [mk(gi, c) for gi in range(8) for c in range(2)])

        def o_pair(br, p):
            def wraw(i, k, a=0, n=HD):
                w = wo32[slot, br, 2 * k:2 * k + 2, (i * HD + a) // 2:(i * HD + a + n) // 2, :]
                return [w[0], w[1]]

            def wsum(i):
                w = ws32[br][:, :, i * 8:(i + 1) * 8, :]
                return [w[c].reshape(HD // 2, 128) for c in range(2)]

            def oraw(k, n):
                o = o32[br][2 * k:2 * k + 2, (2 * p + n) * 64:(2 * p + n + 1) * 64, :]
                return _wide([o[0], o[1]])

            def osum(i):
                o = ot32[(br * 4 + p) % 2][:, :, i * 8:(i + 1) * 8, :]
                return _wide([o[c].reshape(64, 128) for c in range(2)])

            def two(l1, w1, l2, w2, n=HD):
                r1 = jax.lax.dot_general(_wide(l1), w1, NT, preferred_element_type=f32)
                r2 = jax.lax.dot_general(gated(l2, n), w2, NT, preferred_element_type=f32)
                advance(r2, n)
                return r1, r2

            p1, p2 = two(wraw(0, 0), oraw(0, 0), wraw(0, 1), oraw(1, 0))
            c11 = p1 + p2
            done(("w", br), ("o", br * 4 + p))
            p6, p7 = two(wsum(1), osum(1), wsum(2), osum(2))
            u2 = p1 + p6
            u3 = u2 + p7
            p5, p3 = two(wsum(0), osum(0), wsum(3), oraw(1, 1))
            finish_tile(br, 2 * p + 1, _cat([u2 + p5 + p3, u3 + p5], 0))
            p4 = two(wraw(1, 1, 0, HD // 2), osum(3), wraw(1, 1, HD // 2, HD // 2), osum(3), HD // 2)
            finish_tile(br, 2 * p, _cat([c11, u3 - _cat(list(p4), 0)], 0))

        stage_tile(1, MT - 1, jnp.maximum(it - 1, 0) >> 3, acc[D:2 * D, last_tile], it == HKV)

        for u in range(NU):
            plan_vsums(u)
        for br in range(2):
            plan_wsums(br)
            for p in range(4):
                plan_osums(br, p)
        for kind, arg in plan:
            assert st["now"] == tstart[(kind, arg)]
            if kind == "q":
                qb_proj(arg)
            elif kind == "qk":
                qk(arg)
                refill(0, arg)
            elif kind == "o":
                o_single(*arg)
            elif kind == "o2":
                o_pair(*arg)
            else:
                pv(arg)
                if arg != NU - 2:
                    refill(1, arg)
        assert not tasks
        pl.when(more)(lambda: start_wo(slot, nit & 7))
        return carry

    jax.lax.fori_loop(0, NIT, body, 0)

    stage_tile(1, MT - 1, NG - 1, acc[D:2 * D, last_tile], None)
    pltpu.make_async_copy(stage, out_hbm, sems.at[S_OUT]).wait()


@jax.jit
def pallas_concat_heads__gqa_block_cached__gqa_block_cached__near_ridge_kernel(
    A_x: jax.Array,
    A_k_cache: jax.Array,
    A_v_cache: jax.Array,
    A_wq: jax.Array,
    A_wo: jax.Array,
    B_x: jax.Array,
    B_k_cache: jax.Array,
    B_v_cache: jax.Array,
    B_wq: jax.Array,
    B_wo: jax.Array,
):
    any_spec = pl.BlockSpec(memory_space=pl.ANY)
    two = lambda shape, dt: [pltpu.VMEM(shape, dt), pltpu.VMEM(shape, dt)]
    scratch = (
        two((2, 2, 2, GB, SK, 128), bf16)
        + two((M, D), bf16)
        + two((HKV, D, GW), bf16)
        + [pltpu.VMEM((2, 2, 4, D, 128), bf16),
           pltpu.VMEM((HKV, 4, NG, GR, 128), bf16),
           pltpu.VMEM((4, GR, 128), bf16)]
        + two((4, GR, 128), bf16)
        + [pltpu.VMEM((2 * D, GR), f32),
           pltpu.VMEM((M, 2 * D), bf16)]
        + two((2, 4, 9, 7 * 16, 128), bf16)
        + two((32, 64, 128), bf16)
        + two((2, R2, SK), bf16)
        + two((2, 2, SQ, SK), bf16)
        + two((2, 4, R2, 128), f32)
        + two((2, HD // 16, 64, 128), bf16)
        + two((2, 8, 64, 128), bf16)
        + [pltpu.SemaphoreType.DMA((NSEM,))]
    )
    out = pl.pallas_call(
        _kernel,
        in_specs=[any_spec] * 10,
        out_specs=any_spec,
        out_shape=jax.ShapeDtypeStruct((M, 2 * D), bf16),
        scratch_shapes=scratch,
        compiler_params=pltpu.CompilerParams(
            vmem_limit_bytes=120 * 1024 * 1024,
            disable_bounds_checks=True,
            disable_semaphore_checks=True,
        ),
    )(A_x.reshape(M, D), A_k_cache, A_v_cache, A_wq, A_wo.T,
      B_x.reshape(M, D), B_k_cache, B_v_cache, B_wq, B_wo.T)
    return out.reshape(B, SQ, 2 * D)
```

```python
import math

import jax
import jax.numpy as jnp
import jax.experimental.pallas as pl
import jax.experimental.pallas.tpu as pltpu

B, SQ, D = 16, 144, 448
HQ, HKV, SK, DH = 16, 8, 1024, 256
REP = HQ // HKV
GW = REP * DH
SSCALE = (DH ** -0.5) * math.log2(math.e)
NT = (((1,), (1,)), ((), ()))
GB = 8
NG = B // GB
GR = GB * SQ
MT = GR // 128
NU = 2 * GB
NIT = NG * HKV
M = B * SQ
R2 = REP * SQ
CA = 384
HD = D // 2
QB = 2
QPOS = (-1, 0, 10, 12)
OPOS = (2, 4, 6, 8, 16, 11, 14, 15, 16, 16)
MARGIN, ALPHA, LAG, DLAG, DPH, MINGAP = 350, 0.7, 950, 160, 0.1, 12
BLEAD, BMARGIN, BSPAN = 300, 200, 2000
OM, OLEAD, OSPAN = 100, 150, 600
XROWS = (128, 336, 688, 1152)
f32, bf16, u32 = jnp.float32, jnp.bfloat16, jnp.uint32
S_WQ, S_WQB, S_KV, S_WO, S_OUT, S_XB, S_X = 0, 3, 4, 8, 10, 11, 12
NSEM = S_X + len(XROWS)
A11, A12, A22, S1, S2, S3, S4 = range(7)


class _Packed:
    def __init__(self, ref):
        self.ref = ref

    def __getitem__(self, idx):
        nd = len(self.ref.shape)
        idx = list(idx) + [slice(None)] * (nd - len(idx))
        r = idx[nd - 2]
        if r != slice(None):
            idx[nd - 2] = slice(2 * r.start, 2 * r.stop)
        return self.ref.at[tuple(idx)].bitcast(u32)[...]


def _cat(xs, axis):
    return xs[0] if len(xs) == 1 else jnp.concatenate(xs, axis=axis)


def _wide(tiles):
    return _cat([pltpu.bitcast(t, bf16) for t in tiles], 1)


def _lhs_sums(a11, a12, a21, a22):
    s1 = a21 + a22
    s2 = s1 - a11
    return s1, s2, a11 - a21, a12 - s2


def _rhs_sums(b11, b12, b21, b22):
    t1 = b12 - b11
    t2 = b22 - t1
    return t1, t2, b22 - b12, t2 - b21


def _kernel(xa, ka, va, wqa, woa, xb, kb, vb, wqb, wob, out_hbm,
            kbuf, vbuf, xbuf_a, xbuf_b, wqbuf_a, wqbuf_b, wobuf, qbuf_a, qbuf_b, obuf_a, obuf_b,
            acc, stage, abuf0, abuf1, tbuf0, tbuf1, sbuf0, sbuf1, ebuf0, ebuf1, mbuf0, mbuf1,
            wsa, wsb, ot0, ot1, sems):
    kv_hbm = (ka, va, kb, vb)
    wo_hbm = (woa, wob)
    obufs, abufs, tbufs = (obuf_a, obuf_b), (abuf0, abuf1), (tbuf0, tbuf1)
    sbufs, ebufs, mbufs = (sbuf0, sbuf1), (ebuf0, ebuf1), (mbuf0, mbuf1)
    wsbufs, otbufs = (wsa, wsb), (ot0, ot1)
    k32, v32, wo32, qa32, qb32 = (_Packed(r) for r in (kbuf, vbuf, wobuf, qbuf_a, qbuf_b))
    o32, a32, t32, ws32, ot32 = (tuple(_Packed(r) for r in rs)
                                 for rs in (obufs, abufs, tbufs, wsbufs, otbufs))
    last_tile = slice((MT - 1) * 128, MT * 128)

    def wait_all(buf, sem):
        pltpu.make_async_copy(buf, buf, sems.at[sem]).wait()

    def start_kv(slot, i, j, g, h):
        for c in range(2):
            pltpu.make_async_copy(kv_hbm[i].at[g * GB + j, h, :, pl.ds(c * 128, 128)],
                                  (kbuf, vbuf)[i % 2].at[slot, i // 2, c, j],
                                  sems.at[S_KV + 2 * slot + i % 2]).start()

    def start_wo(slot, h):
        for br in range(2):
            for c in range(4):
                col = h * GW + c * 128
                if not isinstance(col, int):
                    col = pl.multiple_of(col, 128)
                pltpu.make_async_copy(wo_hbm[br].at[:, pl.ds(col, 128)], wobuf.at[slot, br, c],
                                      sems.at[S_WO + slot]).start()

    def wqa_copy(h):
        return pltpu.make_async_copy(wqa.at[:, pl.ds(h * GW, GW)], wqbuf_a.at[h],
                                     sems.at[S_WQ + (0 if h == 0 else 1 if h < 4 else 2)])

    xp = []
    r0 = 0
    for n in XROWS:
        xp.append((r0, n))
        r0 += n

    def xa_copy(i):
        r, n = xp[i]
        return pltpu.make_async_copy(xa.at[pl.ds(r, n)], xbuf_a.at[pl.ds(r, n)], sems.at[S_X + i])

    def out_copy(row, br):
        cols = pl.ds(0, CA) if br == 0 else pl.ds(CA, 2 * D - CA)
        return pltpu.make_async_copy(stage.at[pl.ds(row, 128), cols],
                                     out_hbm.at[pl.ds(row, 128), cols], sems.at[S_OUT])

    wqa_copy(0).start()
    for i in range(len(xp) - 1):
        xa_copy(i).start()
    for h in range(1, HKV):
        wqa_copy(h).start()
    xa_copy(len(xp) - 1).start()
    pltpu.make_async_copy(xb, xbuf_b, sems.at[S_XB]).start()
    for h in range(HKV):
        pltpu.make_async_copy(wqb.at[:, pl.ds(h * GW, GW)], wqbuf_b.at[h], sems.at[S_WQB]).start()
    for i0 in range(2):
        for i in range(4):
            for c in range(2):
                pltpu.make_async_copy(kv_hbm[i].at[pl.ds(0, GB), i0, :, pl.ds(c * 128, 128)],
                                      (kbuf, vbuf)[i % 2].at[i0, i // 2, c],
                                      sems.at[S_KV + 2 * i0 + i % 2]).start()
        start_wo(i0, i0)

    def qa_rows(h, gq, r, n):
        row = gq * GR + r
        if not isinstance(row, int):
            row = pl.multiple_of(row, 16)
        q = jnp.dot(xbuf_a[pl.ds(row, n), :], wqbuf_a[h], preferred_element_type=f32)
        for c in range(4):
            qbuf_a[h, c, gq, r:r + n, :] = q[:, c * 128:(c + 1) * 128].astype(bf16)

    acc[CA:2 * D, last_tile] = jnp.zeros((2 * D - CA, 128), f32)
    wqa_copy(0).wait()
    for i in range(len(xp) - 1):
        xa_copy(i).wait()
        qa_rows(0, 0, *xp[i])
    wait_all(wqbuf_a.at[pl.ds(1, 3)], S_WQ + 1)

    def p1_body(i, carry):
        @pl.when(i == 1)
        def _():
            wait_all(wqbuf_a.at[pl.ds(4, HKV - 4)], S_WQ + 2)
            xa_copy(len(xp) - 1).wait()

        for k in range(1, 4):
            idx = 3 * i + k
            qa_rows(idx & 7, idx >> 3, 0, GR)
        return carry

    jax.lax.fori_loop(0, 5, p1_body, 0)
    wait_all(xbuf_b, S_XB)
    wait_all(wqbuf_b, S_WQB)

    def stage_tile(br, t, g, val, cond):
        row = g * GR + t * 128
        if not isinstance(row, int):
            row = pl.multiple_of(row, 128)
        if br == 0:
            stage[pl.ds(row, 128), 0:CA] = val[0:CA].T.astype(bf16)
        else:
            full = jnp.concatenate([acc[CA:D, t * 128:(t + 1) * 128], val], axis=0)
            stage[pl.ds(row, 128), CA:2 * D] = full.T.astype(bf16)
        if cond is None:
            out_copy(row, br).start()
        else:
            @pl.when(cond)
            def _():
                out_copy(row, br).start()

    plan = [("q", i) for i, pos in enumerate(QPOS) if pos == -1] + [("qk", 0)]
    oops = [(k, (br, p)) for br in range(2)
            for k, p in [("o2", 0), ("o2", 1), ("o2", 2), ("o2", 3), ("o", MT - 1)]]
    for u in range(NU + 1):
        if u + 1 < NU:
            plan.append(("qk", u + 1))
        plan += [("q", i) for i, pos in enumerate(QPOS) if pos == u]
        plan += [op for op, pos in zip(oops, OPOS) if pos == u]
        if u < NU:
            plan.append(("pv", u))
    assert plan[-1] == ("o", (1, MT - 1))
    dur = {"q": 4 * QB * SQ, "qk": 4 * R2, "o": D, "o2": 7 * HD // 2, "pv": 7 * SQ}
    tstart, tend = {}, {}
    tt = 0
    for op in plan:
        tstart[op] = tt
        tt += dur[op[0]]
        tend[op] = tt

    for i in range(len(QPOS)):
        assert tend[("q", i)] <= tstart[("qk", GB + QB * i)]

    def body(it, carry):
        g = it >> 3
        h = it & 7
        slot = it & 1
        wait_all(kbuf.at[slot], S_KV + 2 * slot)
        wait_all(vbuf.at[slot], S_KV + 2 * slot + 1)
        wait_all(wobuf.at[slot], S_WO + slot)
        first = h == 0
        last = h == HKV - 1
        always = it >= 0
        zl = it >> 9
        nit = jnp.minimum(it + 2, NIT - 1)
        more = it < NIT - 2
        st = {"now": 0, "free": 0, "seq": 0, "eend": 0}
        tasks = []
        gates = []

        def add_task(key, t, fn):
            st["seq"] += 1
            tasks.append((t, st["seq"], fn, key))

        def done(*keys):
            assert not [x for x in tasks if x[3] in keys], keys

        def spread(key, t_lo, t_hi, fns):
            assert t_lo < t_hi
            for i, fn in enumerate(fns):
                add_task(key, t_lo + (2 * i + 1) * (t_hi - t_lo) // (2 * len(fns)), fn)

        def after(x, tok):
            return jnp.where(always, x, _cat([tok] * (x.shape[0] // 8), 0))

        def gated(tiles, nrows):
            t0 = st["now"]
            mine = [x for x in gates if x[0] < t0 + nrows]
            gates[:] = [x for x in gates if x[0] >= t0 + nrows]
            if mine:
                parts = [tiles[0][r * 8:(r + 1) * 8] for r in range(nrows // 16)]
                for t, mk in mine:
                    r = max(t - t0, 0) // 16
                    parts[r] = jnp.where(always, parts[r], mk)
                tiles = [_cat(parts, 0)] + list(tiles[1:])
            return _wide(tiles)

        def advance(res, nrows):
            t0 = st["now"]
            st["now"] = t0 + nrows
            tasks.sort(key=lambda x: x[:2])
            while tasks:
                t = max(tasks[0][0], st["free"], t0)
                if t >= t0 + nrows:
                    break
                fn = tasks.pop(0)[2]
                st["free"] = t + MINGAP
                r = ((t - t0) // 8) * 8
                fn(res[r:r + 8, 0:128])

        def qb_proj(i):
            n = QB * SQ
            x = xbuf_b[pl.ds(pl.multiple_of(g * GR + i * n, 16), n), :]
            for c in range(4):
                q = jnp.dot(x, wqbuf_b[h, :, c * 128:(c + 1) * 128], preferred_element_type=f32)
                qbuf_b[c, i * n:(i + 1) * n, :] = q.astype(bf16)
                advance(q, n)

        def qk(u):
            br, j = divmod(u, GB)
            rows = slice(j * SQ // 2, (j + 1) * SQ // 2)
            for c in range(4):
                q = qa32[h, :, g, rows, :] if br == 0 else qb32[:, rows, :]
                lhs = gated([_cat([q[d], q[2 + d]], 0) for d in range(2)], R2)
                kw = k32[slot, br, :, j, c * 128:(c + 1) * 128, :]
                s = jax.lax.dot_general(lhs, _wide([kw[0], kw[1]]), NT, preferred_element_type=f32)
                sbufs[u % 2][0, :, c * 256:(c + 1) * 256] = s.astype(bf16)
                mbufs[u % 2][0, c] = jnp.maximum(s[:, :128], s[:, 128:])
                advance(s, R2)
            plan_softmax(u)

        def plan_softmax(u):
            ab, sb, eb, mb = abufs[u % 2], sbufs[u % 2], ebufs[u % 2], mbufs[u % 2]
            t_lo = max(tend[("qk", u)], st["eend"])
            span = tstart[("pv", u)] - MARGIN - t_lo
            rs = {}

            def mke(hd, c):
                def fn(tok):
                    rows = slice(hd * SQ + c * 8, hd * SQ + (c + 1) * 8)
                    pm = mb[zl, :, rows, :]
                    m = jnp.maximum(jnp.maximum(pm[0], pm[1]), jnp.maximum(pm[2], pm[3]))
                    m = jnp.max(m, axis=-1, keepdims=True).astype(bf16).astype(f32)
                    m = after(jnp.broadcast_to(m, (8, 128)), tok)
                    e = jnp.exp2((sb[zl, rows, :].astype(f32) - _cat([m] * 8, 1)) * SSCALE)
                    l = jnp.sum(e, axis=-1, keepdims=True)
                    eb[0, hd, c * 8:(c + 1) * 8, :] = e.astype(bf16)
                    r = pl.reciprocal(l, approx=True)
                    rs[hd, c] = jnp.broadcast_to(r * (2.0 - l * r), (8, 128))
                return fn

            def mkd(gi, k, t):
                def fn(tok):
                    e = eb[zl, :, gi * 16:(gi + 1) * 16, k * 256:(k + 1) * 256].astype(f32)
                    r0 = _cat([rs[0, 2 * gi], rs[0, 2 * gi + 1]], 0)
                    r1 = after(_cat([rs[1, 2 * gi], rs[1, 2 * gi + 1]], 0), tok)
                    a11, a12 = e[0, :, :128] * r0, e[0, :, 128:] * r0
                    a21, a22 = e[1, :, :128] * r1, e[1, :, 128:] * r1
                    ab[0, k, gi] = _cat([a11, a12, a22, *_lhs_sums(a11, a12, a21, a22)], 0).astype(bf16)
                    if k == 3:
                        gates.append((t + LAG, a32[u % 2][zl, 0, 0, 0:8, :]))
                return fn

            nd = 1
            while (nd - DPH) * span / (38.0 + nd) < DLAG:
                nd += 1
            step = span / (38.0 + nd)
            if u + 1 < NU and t_lo + 36 * step > tend[("qk", u + 1)]:
                nq = tend[("qk", u + 1)]
                step = (nq + ALPHA * (t_lo + 36 * step - nq) - t_lo) / 36.0
                nd = 1
                while (nd - DPH) * step < DLAG:
                    nd += 1
            st["eend"] = int(t_lo + 36 * step)
            i = 0
            for gi in range(9):
                for hd in range(2):
                    for half in range(2):
                        add_task(("p", u), t_lo + int(i * step), mke(hd, gi * 2 + half))
                        i += 1
                for k in range(4):
                    t = t_lo + int((i - 1 + k + nd - DPH) * step)
                    add_task(("p", u), t, mkd(gi, k, t))

        def plan_vsums(u):
            br, j = divmod(u, GB)

            def mk(bi):
                def fn(tok):
                    r = (bi // 8) * 256 + (bi % 8) * 16
                    v1 = vbuf[slot, br, :, j, r:r + 16, :].astype(f32)
                    v2 = vbuf[slot, br, :, j, r + 128:r + 144, :].astype(f32)
                    tbufs[u % 2][bi] = _cat(list(_rhs_sums(v1[0], after(v1[1], tok), v2[0], v2[1])), 0).astype(bf16)
                return fn
            t_lo = tend[("pv", u - 2)] + BLEAD if u >= 2 else (0 if u == 0 else tstart[("qk", 0)])
            spread(("v", u), t_lo, min(tstart[("pv", u)] - BMARGIN, t_lo + BSPAN), [mk(bi) for bi in range(32)])

        def refill(kv, u):
            pl.when(more)(lambda: start_kv(slot, 2 * (u // GB) + kv, u % GB, nit >> 3, nit & 7))

        def pv(u):
            br, j = divmod(u, GB)

            def vraw(kh, n):
                v = v32[slot, br, n, j]
                return pltpu.bitcast(_cat([v[k * 128 + kh * 64:k * 128 + (kh + 1) * 64] for k in range(4)], 0), bf16)

            def vsum(i):
                return pltpu.bitcast(t32[u % 2][:, i * 8:(i + 1) * 8, :].reshape(256, 128), bf16)

            def mm(op, w):
                a = a32[u % 2][0, :, :, op * 8:(op + 1) * 8, :]
                r = jnp.dot(gated([a[k].reshape(SQ // 2, 128) for k in range(4)], SQ), w,
                            preferred_element_type=f32)
                advance(r, SQ)
                return r

            rows = slice(j * SQ, (j + 1) * SQ)
            done(("p", u), ("v", u))
            p1 = mm(A11, vraw(0, 0))
            p2 = mm(A12, vraw(1, 0))
            obufs[br][0, rows, :] = (p1 + p2).astype(bf16)
            u2 = p1 + mm(S2, vsum(1))
            u3 = u2 + mm(S3, vsum(2))
            p5 = mm(S1, vsum(0))
            u4 = u2 + p5
            obufs[br][3, rows, :] = (u3 + p5).astype(bf16)
            if u == NU - 1:
                refill(1, u - 1)
            obufs[br][1, rows, :] = (u4 + mm(S4, vraw(1, 1))).astype(bf16)
            obufs[br][2, rows, :] = (u3 - mm(A22, vsum(3))).astype(bf16)

        def finish_tile(br, t, r):
            old = acc[br * D:(br + 1) * D, t * 128:(t + 1) * 128]
            new = jnp.where(first, 0.0, old) + r
            acc[br * D:(br + 1) * D, t * 128:(t + 1) * 128] = new
            if not (br == 1 and t == MT - 1):
                stage_tile(br, t, g, new, last)

        def o_single(br, t):
            w = wo32[slot, br]
            o = o32[br][:, t * 64:(t + 1) * 64, :]
            r = jax.lax.dot_general(gated([w[c] for c in range(4)], D), _wide([o[c] for c in range(4)]), NT,
                                    preferred_element_type=f32)
            finish_tile(br, t, r)
            advance(r, D)

        def plan_wsums(br):
            def mk(gi, c):
                def fn(tok):
                    w1 = wobuf[slot, br, :, gi * 16:(gi + 1) * 16, :].astype(f32)
                    w2 = wobuf[slot, br, :, HD + gi * 16:HD + (gi + 1) * 16, :].astype(f32)
                    wsbufs[br][c, gi] = _cat(list(_lhs_sums(w1[c], w1[2 + c], after(w2[c], tok), w2[2 + c])),
                                             0).astype(bf16)
                return fn
            spread(("w", br), br * 1150, (br + 1) * 1150, [mk(gi, c) for gi in range(HD // 16) for c in range(2)])

        def plan_osums(br, p):
            idx = br * 4 + p

            def mk(gi, c):
                def fn(tok):
                    r = 2 * p * 128 + gi * 16
                    o1 = obufs[br][:, r:r + 16, :].astype(f32)
                    o2 = obufs[br][:, r + 128:r + 144, :].astype(f32)
                    otbufs[idx % 2][c, gi] = _cat(list(_rhs_sums(o1[c], after(o2[c], tok), o1[2 + c], o2[2 + c])),
                                                  0).astype(bf16)
                return fn
            t_hi = tstart[("o2", (br, p))] - OM
            t_lo = max(tend[("pv", br * GB + 2 * p + 1)] + OLEAD, t_hi - OSPAN)
            if idx >= 2:
                t_lo = max(t_lo, tend[("o2", divmod(idx - 2, 4))])
            spread(("o", idx), t_lo, t_hi, [mk(gi, c) for gi in range(8) for c in range(2)])

        def o_pair(br, p):
            def wraw(i, k, a=0, n=HD):
                w = wo32[slot, br, 2 * k:2 * k + 2, (i * HD + a) // 2:(i * HD + a + n) // 2, :]
                return [w[0], w[1]]

            def wsum(i):
                w = ws32[br][:, :, i * 8:(i + 1) * 8, :]
                return [w[c].reshape(HD // 2, 128) for c in range(2)]

            def oraw(k, n):
                o = o32[br][2 * k:2 * k + 2, (2 * p + n) * 64:(2 * p + n + 1) * 64, :]
                return _wide([o[0], o[1]])

            def osum(i):
                o = ot32[(br * 4 + p) % 2][:, :, i * 8:(i + 1) * 8, :]
                return _wide([o[c].reshape(64, 128) for c in range(2)])

            def two(l1, w1, l2, w2, n=HD):
                r1 = jax.lax.dot_general(_wide(l1), w1, NT, preferred_element_type=f32)
                r2 = jax.lax.dot_general(gated(l2, n), w2, NT, preferred_element_type=f32)
                advance(r2, n)
                return r1, r2

            p1, p2 = two(wraw(0, 0), oraw(0, 0), wraw(0, 1), oraw(1, 0))
            c11 = p1 + p2
            done(("w", br), ("o", br * 4 + p))
            p6, p7 = two(wsum(1), osum(1), wsum(2), osum(2))
            u2 = p1 + p6
            u3 = u2 + p7
            p5, p3 = two(wsum(0), osum(0), wsum(3), oraw(1, 1))
            finish_tile(br, 2 * p + 1, _cat([u2 + p5 + p3, u3 + p5], 0))
            p4 = two(wraw(1, 1, 0, HD // 2), osum(3), wraw(1, 1, HD // 2, HD // 2), osum(3), HD // 2)
            finish_tile(br, 2 * p, _cat([c11, u3 - _cat(list(p4), 0)], 0))

        stage_tile(1, MT - 1, jnp.maximum(it - 1, 0) >> 3, acc[D:2 * D, last_tile], it == HKV)

        for u in range(NU):
            plan_vsums(u)
        for br in range(2):
            plan_wsums(br)
            for p in range(4):
                plan_osums(br, p)
        for kind, arg in plan:
            assert st["now"] == tstart[(kind, arg)]
            if kind == "q":
                qb_proj(arg)
            elif kind == "qk":
                qk(arg)
                refill(0, arg)
            elif kind == "o":
                o_single(*arg)
            elif kind == "o2":
                o_pair(*arg)
            else:
                pv(arg)
                if arg != NU - 2:
                    refill(1, arg)
        assert not tasks
        pl.when(more)(lambda: start_wo(slot, nit & 7))
        return carry

    jax.lax.fori_loop(0, NIT, body, 0)

    stage_tile(1, MT - 1, NG - 1, acc[D:2 * D, last_tile], None)
    pltpu.make_async_copy(stage, out_hbm, sems.at[S_OUT]).wait()


@jax.jit
def pallas_concat_heads__gqa_block_cached__gqa_block_cached__near_ridge_kernel(
    A_x: jax.Array,
    A_k_cache: jax.Array,
    A_v_cache: jax.Array,
    A_wq: jax.Array,
    A_wo: jax.Array,
    B_x: jax.Array,
    B_k_cache: jax.Array,
    B_v_cache: jax.Array,
    B_wq: jax.Array,
    B_wo: jax.Array,
):
    any_spec = pl.BlockSpec(memory_space=pl.ANY)
    two = lambda shape, dt: [pltpu.VMEM(shape, dt), pltpu.VMEM(shape, dt)]
    scratch = (
        two((2, 2, 2, GB, SK, 128), bf16)
        + two((M, D), bf16)
        + two((HKV, D, GW), bf16)
        + [pltpu.VMEM((2, 2, 4, D, 128), bf16),
           pltpu.VMEM((HKV, 4, NG, GR, 128), bf16),
           pltpu.VMEM((4, GR, 128), bf16)]
        + two((4, GR, 128), bf16)
        + [pltpu.VMEM((2 * D, GR), f32),
           pltpu.VMEM((M, 2 * D), bf16)]
        + two((2, 4, 9, 7 * 16, 128), bf16)
        + two((32, 64, 128), bf16)
        + two((2, R2, SK), bf16)
        + two((2, 2, SQ, SK), bf16)
        + two((2, 4, R2, 128), f32)
        + two((2, HD // 16, 64, 128), bf16)
        + two((2, 8, 64, 128), bf16)
        + [pltpu.SemaphoreType.DMA((NSEM,))]
    )
    out = pl.pallas_call(
        _kernel,
        in_specs=[any_spec] * 10,
        out_specs=any_spec,
        out_shape=jax.ShapeDtypeStruct((M, 2 * D), bf16),
        scratch_shapes=scratch,
        compiler_params=pltpu.CompilerParams(
            vmem_limit_bytes=120 * 1024 * 1024,
            disable_bounds_checks=True,
            disable_semaphore_checks=True,
        ),
    )(A_x.reshape(M, D), A_k_cache, A_v_cache, A_wq, A_wo.T,
      B_x.reshape(M, D), B_k_cache, B_v_cache, B_wq, B_wo.T)
    return out.reshape(B, SQ, 2 * D)
```
